```python
import jax
import jax.numpy as jnp

def _softmax(x, axis=-1):
    return jax.nn.softmax(x, axis=axis)

def _gelu(x):
    return jax.nn.gelu(x, approximate=True)

def _silu(x):
    return jax.nn.silu(x)

def _sigmoid(x):
    return jax.nn.sigmoid(x)

def _layernorm(x, axis=-1, eps=1e-05):
    m = jnp.mean(x, axis=axis, keepdims=True)
    v = jnp.var(x, axis=axis, keepdims=True)
    return (x - m) / jnp.sqrt(v + eps)

def _scatter_add(tgt, idx, src, axis=0):
    return tgt.at[idx].add(src)

def _segment_sum(src, seg, n):
    return jax.ops.segment_sum(src, seg, n)

class _Rng:

    def __init__(self, key):
        self._k = key

    def _next(self):
        self._k, sub = jax.random.split(self._k)
        return sub

    def normal(self, shape):
        return jax.random.normal(self._next(), shape, dtype=jnp.bfloat16)

    def randint(self, lo, hi, shape):
        return jax.random.randint(self._next(), shape, lo, hi, dtype=jnp.int32)

    def uniform(self, shape, lo=0.0, hi=1.0):
        return jax.random.uniform(self._next(), shape, jnp.bfloat16, lo, hi)

    def permutation(self, n):
        return jax.random.permutation(self._next(), n)
kernel_name = 'adaLN_cond__sliding_block_cached__glu_gated_bilinear__decode'

def setup_inputs():
    _rng = _Rng(jax.random.key(int.from_bytes(__import__("os").urandom(4), "little")))
    _w = lambda a: (lambda t: t.astype(jnp.bfloat16) if jnp.issubdtype(t.dtype, jnp.floating) else t)(jnp.asarray(a))

    def _A_setup():
        B, Sq, D = (1, 1, 640)
        Hq, Hkv, Sk, Dh = (32, 32, 32768, 192)
        assert Hq % Hkv == 0, (Hq, Hkv)
        return {'x': _w((lambda *s: _rng.normal(s) * 0.05)(B, Sq, D)), 'k_cache': _w((lambda *s: _rng.normal(s) * 0.05)(B, Hkv, Sk, Dh)), 'v_cache': _w((lambda *s: _rng.normal(s) * 0.05)(B, Hkv, Sk, Dh)), 'wq': _w((lambda *s: _rng.normal(s) * 0.05)(D, Hq * Dh) * D ** (-0.5)), 'wo': _w((lambda *s: _rng.normal(s) * 0.05)(Hq * Dh, D) * (Hq * Dh) ** (-0.5))}
    _A_in = _A_setup()

    def _B_setup():
        B, S, D, F = (1, 1, 640, 1536)
        return {'x': _w((lambda *s: _rng.normal(s) * 0.05)(B, S, D)), 'w_gate': _w((lambda *s: _rng.normal(s) * 0.05)(D, F) * D ** (-0.5)), 'w_up': _w((lambda *s: _rng.normal(s) * 0.05)(D, F) * D ** (-0.5)), 'w_down': _w((lambda *s: _rng.normal(s) * 0.05)(F, D) * F ** (-0.5))}
    _B_in = _B_setup()
    return {'A_x': _A_in['x'], 'A_k_cache': _A_in['k_cache'], 'A_v_cache': _A_in['v_cache'], 'A_wq': _A_in['wq'], 'A_wo': _A_in['wo'], 'B_x': _B_in['x'], 'B_w_gate': _B_in['w_gate'], 'B_w_up': _B_in['w_up'], 'B_w_down': _B_in['w_down'], 'c': _w((lambda *s: _rng.normal(s) * 0.05)(1, 640)), 'w_mod': _w((lambda *s: _rng.normal(s) * 0.05)(640, 6 * 640) * 640 ** (-0.5))}

def reference(A_x, A_k_cache, A_v_cache, A_wq, A_wo, B_x, B_w_gate, B_w_up, B_w_down, c, w_mod):

    def _A_ref(x, k_cache, v_cache, wq, wo):
        B, Sq, D = x.shape
        Hq, Dh = (32, 192)
        Hkv, Sk = (k_cache.shape[1], k_cache.shape[2])
        W = min(4096, max(256, Sk // 4))
        rep = Hq // Hkv
        q = (lambda x, *d: x.transpose(*d))((x @ wq).reshape(B, Sq, Hq, Dh), 0, 2, 1, 3)
        k = jnp.repeat(k_cache[:, :, Sk - W:, :], rep, axis=1)
        v = jnp.repeat(v_cache[:, :, Sk - W:, :], rep, axis=1)
        scores = jnp.einsum('bhqd,bhkd->bhqk', q, k) * Dh ** (-0.5)
        p = _softmax(scores, axis=-1)
        o = jnp.einsum('bhqk,bhkd->bhqd', p, v)
        return (lambda x, *d: x.transpose(*d))(o, 0, 2, 1, 3).reshape(B, Sq, Hq * Dh) @ wo

    def _B_ref(x, w_gate, w_up, w_down):
        g = jnp.einsum('bsd,df->bsf', x, w_gate)
        u = jnp.einsum('bsd,df->bsf', x, w_up)
        h = g * u
        return jnp.einsum('bsf,fd->bsd', h, w_down)
    x = A_x
    mod = (_silu(c) @ w_mod).reshape(c.shape[0], 6, 1, -1)
    sa, ca, ga, sb, cb, gb = (mod[:, 0].copy(), mod[:, 1].copy(), mod[:, 2].copy(), mod[:, 3].copy(), mod[:, 4].copy(), mod[:, 5].copy())
    h = _layernorm(x, axis=-1) * (1 + ca) + sa
    x = x + ga * _A_ref(h, A_k_cache, A_v_cache, A_wq, A_wo)
    h = _layernorm(x, axis=-1) * (1 + cb) + sb
    x = x + gb * _B_ref(h, B_w_gate, B_w_up, B_w_down)
    return x
```

```python
import jax
import jax.numpy as jnp
from jax import lax
import jax.experimental.pallas as pl
import jax.experimental.pallas.tpu as pltpu

D = 640
HQ = 32
DH = 192
ROWS = HQ * DH
F = 1536
GH = 8
GROWS = GH * DH
NG = HQ // GH
EPS = 1e-5


def _layernorm(x):
    m = jnp.mean(x, axis=-1, keepdims=True)
    xc = x - m
    v = jnp.mean(xc * xc, axis=-1, keepdims=True)
    return xc * lax.rsqrt(v + EPS)


def make_kernel(SK, W, R, NBUF, FCH):
    NCH = ROWS // R
    CPG = GROWS // R
    NF = F // FCH
    C0 = SK - W
    scale = DH ** -0.5

    def kernel(x_hbm, c_hbm, wmod_hbm, wq_hbm, kt_hbm, vt_hbm, wo_hbm, wg_hbm, wu_hbm, wd_hbm,
               out_ref,
               x_v, c_v, wmod_v, wq_v, wo_v, wg_v, wu_v, wd_v, kv, qbd, s_ref, p_ref, linv_ref,
               sem_kv, sem_w, sem_f):
        def kv_copy(src, c, slot):
            r0 = c * R
            if not isinstance(r0, int):
                r0 = pl.multiple_of(r0, R)
            return pltpu.make_async_copy(src.at[pl.ds(r0, R), pl.ds(C0, W)], kv.at[slot], sem_kv.at[slot])

        cp_x = pltpu.make_async_copy(x_hbm, x_v, sem_w.at[0])
        cp_c = pltpu.make_async_copy(c_hbm, c_v, sem_w.at[1])
        cp_ma = pltpu.make_async_copy(wmod_hbm.at[:, pl.ds(0, 2 * D)], wmod_v.at[:, pl.ds(0, 2 * D)], sem_w.at[2])
        cp_mb = pltpu.make_async_copy(wmod_hbm.at[:, pl.ds(2 * D, 4 * D)], wmod_v.at[:, pl.ds(2 * D, 4 * D)], sem_w.at[3])
        cp_wq = pltpu.make_async_copy(wq_hbm, wq_v, sem_w.at[4])
        cp_wo = pltpu.make_async_copy(wo_hbm, wo_v, sem_w.at[5])

        def ffn_copies(j):
            return (
                pltpu.make_async_copy(wg_hbm.at[:, pl.ds(j * FCH, FCH)], wg_v.at[:, pl.ds(j * FCH, FCH)], sem_f.at[3 * j]),
                pltpu.make_async_copy(wu_hbm.at[:, pl.ds(j * FCH, FCH)], wu_v.at[:, pl.ds(j * FCH, FCH)], sem_f.at[3 * j + 1]),
                pltpu.make_async_copy(wd_hbm.at[pl.ds(j * FCH, FCH), :], wd_v.at[pl.ds(j * FCH, FCH), :], sem_f.at[3 * j + 2]),
            )

        cp_c.start()
        cp_x.start()
        cp_ma.start()
        cp_wq.start()
        for j in range(NBUF):
            kv_copy(kt_hbm, j, j).start()
        cp_mb.start()

        cp_c.wait()
        cp_x.wait()
        c32 = jnp.broadcast_to(c_v[...].astype(jnp.float32), (8, D))
        sc = (c32 * jax.nn.sigmoid(c32)).astype(jnp.bfloat16)
        x32 = jnp.broadcast_to(x_v[...].astype(jnp.float32), (8, D))
        ln1 = _layernorm(x32)
        cp_ma.wait()
        mod_a = jnp.dot(sc, wmod_v[:, 0:2 * D], preferred_element_type=jnp.float32)
        h = (ln1 * (1.0 + mod_a[:, D:2 * D]) + mod_a[:, 0:D]).astype(jnp.bfloat16)
        cp_wq.wait()
        row = lax.broadcasted_iota(jnp.int32, (8, R), 0)
        col = lax.broadcasted_iota(jnp.int32, (8, R), 1)
        for c in range(NCH):
            q = jnp.dot(h, wq_v[:, c * R:(c + 1) * R], preferred_element_type=jnp.float32)
            gcol = col + (c % CPG) * R
            mask = (gcol >= row * DH) & (gcol < (row + 1) * DH)
            qbd[c] = jnp.where(mask, q, 0.0).astype(jnp.bfloat16)

        def issue_next(t, slot):
            nxt = t + NBUF

            @pl.when(nxt < NCH)
            def _():
                kv_copy(kt_hbm, nxt, slot).start()

            @pl.when(nxt == NCH)
            def _():
                cp_wo.start()

            @pl.when(jnp.logical_and(nxt >= NCH, nxt < 2 * NCH))
            def _():
                kv_copy(vt_hbm, nxt - NCH, slot).start()

            @pl.when(nxt == 2 * NCH - 1)
            def _():
                for j in range(NF):
                    for cp in ffn_copies(j):
                        cp.start()

        def k_body(t, carry):
            slot = t % NBUF
            kv_copy(kt_hbm, t, slot).wait()
            s = jnp.dot(qbd[t], kv[slot], preferred_element_type=jnp.float32)
            j = t % CPG

            @pl.when(j == 0)
            def _():
                s_ref[...] = s

            @pl.when(j != 0)
            def _():
                s_ref[...] += s

            issue_next(t, slot)

            @pl.when(j == CPG - 1)
            def _():
                g = t // CPG
                sg = s_ref[...] * scale
                m = jnp.max(sg, axis=-1, keepdims=True)
                e = jnp.exp(sg - m)
                l = jnp.sum(e, axis=-1, keepdims=True)
                p_ref[g] = e.astype(jnp.bfloat16)
                linv_ref[g] = jnp.broadcast_to(1.0 / l, (8, 128))
            return carry

        lax.fori_loop(0, NCH, k_body, 0)

        cp_mb.wait()
        mod_b = jnp.dot(sc, wmod_v[:, 2 * D:6 * D], preferred_element_type=jnp.float32)
        cp_wo.wait()

        def v_body(u, acc):
            t = u + NCH
            slot = t % NBUF
            kv_copy(vt_hbm, u, slot).wait()
            g = u // CPG
            o = lax.dot_general(p_ref[g], kv[slot], (((1,), (1,)), ((), ())),
                                preferred_element_type=jnp.float32)
            issue_next(t, slot)
            gcol = col + (u % CPG) * R
            mask = (gcol >= row * DH) & (gcol < (row + 1) * DH)
            o = jnp.where(mask, o * linv_ref[g][:, 0:1], 0.0).astype(jnp.bfloat16)
            r0 = pl.multiple_of(u * R, R)
            return acc + jnp.dot(o, wo_v[pl.ds(r0, R), :], preferred_element_type=jnp.float32)

        acc = lax.fori_loop(0, NCH, v_body, jnp.zeros((8, D), jnp.float32))
        attn = jnp.broadcast_to(jnp.sum(acc, axis=0, keepdims=True), (8, D))

        x1 = x32 + mod_b[:, 0:D] * attn
        h2 = (_layernorm(x1) * (1.0 + mod_b[:, 2 * D:3 * D]) + mod_b[:, D:2 * D]).astype(jnp.bfloat16)
        y = jnp.zeros((8, D), jnp.float32)
        for j in range(NF):
            cg, cu, cd = ffn_copies(j)
            cg.wait()
            gg = jnp.dot(h2, wg_v[:, j * FCH:(j + 1) * FCH], preferred_element_type=jnp.float32)
            cu.wait()
            uu = jnp.dot(h2, wu_v[:, j * FCH:(j + 1) * FCH], preferred_element_type=jnp.float32)
            hh = (gg * uu).astype(jnp.bfloat16)
            cd.wait()
            y = y + jnp.dot(hh, wd_v[j * FCH:(j + 1) * FCH, :], preferred_element_type=jnp.float32)
        out = x1 + mod_b[:, 3 * D:4 * D] * y
        out_ref[...] = out[0:1, :].astype(out_ref.dtype)

    scratch = [
        pltpu.VMEM((1, D), jnp.bfloat16),
        pltpu.VMEM((1, D), jnp.bfloat16),
        pltpu.VMEM((D, 6 * D), jnp.bfloat16),
        pltpu.VMEM((D, ROWS), jnp.bfloat16),
        pltpu.VMEM((ROWS, D), jnp.bfloat16),
        pltpu.VMEM((D, F), jnp.bfloat16),
        pltpu.VMEM((D, F), jnp.bfloat16),
        pltpu.VMEM((F, D), jnp.bfloat16),
        pltpu.VMEM((NBUF, R, W), jnp.bfloat16),
        pltpu.VMEM((NCH, 8, R), jnp.bfloat16),
        pltpu.VMEM((8, W), jnp.float32),
        pltpu.VMEM((NG, 8, W), jnp.bfloat16),
        pltpu.VMEM((NG, 8, 128), jnp.float32),
        pltpu.SemaphoreType.DMA((NBUF,)),
        pltpu.SemaphoreType.DMA((6,)),
        pltpu.SemaphoreType.DMA((3 * NF,)),
    ]
    return kernel, scratch


@jax.jit
def pallas_adaLN_cond__sliding_block_cached__glu_gated_bilinear__decode_kernel(
    A_x: jax.Array,
    A_k_cache: jax.Array,
    A_v_cache: jax.Array,
    A_wq: jax.Array,
    A_wo: jax.Array,
    B_x: jax.Array,
    B_w_gate: jax.Array,
    B_w_up: jax.Array,
    B_w_down: jax.Array,
    c: jax.Array,
    w_mod: jax.Array,
):
    R, NBUF, FCH = 384, 4, 512
    SK = A_k_cache.shape[2]
    W = min(4096, max(256, SK // 4))
    kt = jnp.swapaxes(A_k_cache, 2, 3).reshape(ROWS, SK)
    vt = jnp.swapaxes(A_v_cache, 2, 3).reshape(ROWS, SK)
    kernel, scratch = make_kernel(SK, W, R, NBUF, FCH)
    out = pl.pallas_call(
        kernel,
        in_specs=[pl.BlockSpec(memory_space=pl.ANY)] * 10,
        out_specs=pl.BlockSpec(memory_space=pltpu.VMEM),
        out_shape=jax.ShapeDtypeStruct((1, D), jnp.bfloat16),
        scratch_shapes=scratch,
        compiler_params=pltpu.CompilerParams(vmem_limit_bytes=100 * 1024 * 1024),
    )(A_x.reshape(1, D), c, w_mod, A_wq, kt, vt, A_wo, B_w_gate, B_w_up, B_w_down)
    return out.reshape(1, 1, D)
```

```python
import jax
import jax.numpy as jnp
from jax import lax
import jax.experimental.pallas as pl
import jax.experimental.pallas.tpu as pltpu

D = 640
HQ = 32
DH = 192
ROWS = HQ * DH
F = 1536
GH = 8
GROWS = GH * DH
NG = HQ // GH
BR = 128
NBLK = ROWS // BR
BPG = GROWS // BR
EPS = 1e-5
HI, LO = 0, 1


def _layernorm(x):
    m = jnp.mean(x, axis=-1, keepdims=True)
    xc = x - m
    v = jnp.mean(xc * xc, axis=-1, keepdims=True)
    return xc * lax.rsqrt(v + EPS)


def _static(i):
    return isinstance(i, int)


def _mult(i, m):
    return i if _static(i) else pl.multiple_of(i, m)


def _when(cond, fn):
    if isinstance(cond, bool):
        if cond:
            fn()
    else:
        pl.when(cond)(fn)


def make_kernel(SK, W, Rt=128, Wt=1024, LA=3, NB=8, QR=64, QC=2048, every=4, NS=100, S=4,
                TL=4, mb_rows=8, mb_cols=1280, wd_chunks=(1024, 384, 128), trickle=True):
    C0 = SK - W
    scale = DH ** -0.5
    nr, nc = BR // Rt, W // Wt
    n = nr * nc
    CW = W // n
    NQR, NQC = D // QR, ROWS // QC
    NI = NQR * NQC
    NSTEP = NI + 2 * NBLK * n
    wo_rows = BR // n
    assert NB >= LA + 2 and TL <= n and sum(wd_chunks) == F
    n_mb = (D // mb_rows) * (4 * D // mb_cols)
    n_gu = 2 * (D // 8) - NS
    t_mb0 = 0
    t_gu0 = t_mb0 + n_mb
    t_wo0 = NI + NBLK * n
    assert t_gu0 + n_gu <= t_wo0, (t_gu0, n_gu, t_wo0)
    assert (NS + 1) * every <= NSTEP and NS >= D // 8
    TR = 2 * TL
    o_kv = 0
    o_tr = o_kv + NB * n
    o_s1 = o_tr + TR
    o_s2 = o_s1 + S
    o_wq = o_s2 + S
    o_misc = o_wq + NI
    o_wd = o_misc + 3
    NSEM = o_wd + len(wd_chunks)

    def kernel(x_hbm, c_hbm, wmod_hbm, wq_hbm, kt_hbm, vt_hbm, wo_hbm, wg_hbm, wu_hbm, wd_hbm,
               out_ref,
               x_v, c_v, wma_v, wmb_v, wq_v, wo_v, wg_v, wu_v, wd_v, kv, qbd, s_ref, p_ref, linv_ref,
               stage, sems):
        def kv_copy(src, b, slot, j):
            rj, cj = j // nc, j % nc
            r0 = _mult(b * BR + rj * Rt, Rt)
            return pltpu.make_async_copy(
                src.at[pl.ds(r0, Rt), pl.ds(C0 + cj * Wt, Wt)],
                kv.at[slot, pl.ds(rj * Rt, Rt), pl.ds(cj * Wt, Wt)],
                sems.at[o_kv + slot * n + j])

        def wq_copy(u):
            cg, r = u // NQR, u % NQR
            return pltpu.make_async_copy(
                wq_hbm.at[pl.ds(r * QR, QR), pl.ds(cg * QC, QC)],
                wq_v.at[pl.ds(r * QR, QR), pl.ds(cg * QC, QC)], sems.at[o_wq + u])

        def mb_copy(t):
            i = t - t_mb0
            ncol = 4 * D // mb_cols
            r0 = _mult((i // ncol) * mb_rows, 8)
            c0 = _mult((i % ncol) * mb_cols, 128)
            return pltpu.make_async_copy(
                wmod_hbm.at[pl.ds(r0, mb_rows), pl.ds(_mult(2 * D + c0, 128), mb_cols)],
                wmb_v.at[pl.ds(r0, mb_rows), pl.ds(c0, mb_cols)], sems.at[o_tr + t % TR])

        def gu_copy(t):
            r0 = _mult((t - t_gu0 + NS - D // 8) * 8, 8)
            return pltpu.make_async_copy(wu_hbm.at[pl.ds(r0, 8)], wu_v.at[pl.ds(r0, 8)],
                                         sems.at[o_tr + t % TR])

        def wo_copy(t):
            r0 = _mult((t - t_wo0) * wo_rows, wo_rows)
            return pltpu.make_async_copy(wo_hbm.at[pl.ds(r0, wo_rows)], wo_v.at[pl.ds(r0, wo_rows)],
                                         sems.at[o_tr + t % TR])

        segs = [(mb_copy, t_mb0, t_mb0 + n_mb), (gu_copy, t_gu0, t_gu0 + n_gu), (wo_copy, t_wo0, NSTEP)]

        def trickle_op(t, lo, hi, op):
            for mk, a, b in segs:
                if b <= a or b <= lo or a > hi:
                    continue
                if _static(t):
                    cond = a <= t < b
                elif a <= lo and hi < b:
                    cond = True
                elif a <= lo:
                    cond = t < b
                elif hi < b:
                    cond = t >= a
                else:
                    cond = jnp.logical_and(t >= a, t < b)
                _when(cond, lambda mk=mk: op(mk(t)))

        def hop1(src, i, j):
            r0 = _mult(i * 8, 8)
            return pltpu.make_async_copy(src.at[pl.ds(r0, 8)], stage.at[j % S], sems.at[o_s1 + j % S])

        def hop2(dst, i, j):
            r0 = _mult(i * 8, 8)
            return pltpu.make_async_copy(stage.at[j % S], dst.at[pl.ds(r0, 8)], sems.at[o_s2 + j % S])

        NP = D // 8

        def s_op(j, hop, op):
            a, b = (wg_hbm, wu_hbm) if hop is hop1 else (wg_v, wu_v)
            _when(j < NP, lambda: op(hop(a, j, j)))
            _when(j >= NP, lambda: op(hop(b, j - NP, j)))

        start_hi = lambda cp: cp.start(priority=HI)
        start_lo = lambda cp: cp.start(priority=LO)
        wait = lambda cp: cp.wait()

        def smem_tick(j):
            def a():
                s_op(j, hop1, wait)
                s_op(j, hop2, start_hi)
            _when(j < NS, a)
            _when((j >= 1) & (j <= NS) if not _static(j) else (1 <= j <= NS), lambda: s_op(j - 1, hop2, wait))
            _when(j + S - 1 < NS, lambda: s_op(j + S - 1, hop1, start_hi))

        def side_traffic(u, lo, hi):
            trickle_op(u, lo, hi, start_hi)
            if _static(u):
                if u >= TL:
                    trickle_op(u - TL, lo - TL, hi - TL, wait)
            else:
                trickle_op(u - TL, lo - TL, hi - TL, wait)
            _when(u % every == every - 1, lambda: smem_tick(u // every))

        wd_cps = []
        r = 0
        for i, rows in enumerate(wd_chunks):
            wd_cps.append(pltpu.make_async_copy(wd_hbm.at[pl.ds(r, rows)], wd_v.at[pl.ds(r, rows)],
                                                sems.at[o_wd + i]))
            r += rows

        def kv_step(tau, j, lo, hi):
            slot = tau % NB
            kv_copy(kt_hbm, 0, slot, j).wait()
            nxt = tau + LA
            nslot = nxt % NB
            u = NI + tau * n + j
            side_traffic(u, NI + lo * n + j, NI + hi * n + j)
            if lo + LA < NBLK:
                _when(True if hi + LA < NBLK else nxt < NBLK,
                      lambda: start_lo(kv_copy(kt_hbm, nxt, nslot, j)))
            if hi + LA >= NBLK and lo + LA < 2 * NBLK:
                c1 = True if lo + LA >= NBLK else nxt >= NBLK
                c2 = True if hi + LA < 2 * NBLK else nxt < 2 * NBLK
                cond = c2 if c1 is True else (c1 if c2 is True else jnp.logical_and(c1, c2))
                _when(cond, lambda: start_lo(kv_copy(vt_hbm, nxt - NBLK, nslot, j)))
            if j == n - 1 and lo + LA <= 2 * NBLK - 1 <= hi + LA:
                def tail():
                    for cp in wd_cps:
                        start_lo(cp)
                _when(nxt == 2 * NBLK - 1, tail)

        cp_c = pltpu.make_async_copy(c_hbm, c_v, sems.at[o_misc])
        cp_x = pltpu.make_async_copy(x_hbm, x_v, sems.at[o_misc + 1])
        cp_ma = pltpu.make_async_copy(wmod_hbm.at[:, pl.ds(0, 2 * D)], wma_v, sems.at[o_misc + 2])

        start_hi(cp_c)
        start_hi(cp_x)
        start_hi(cp_ma)
        for u in range(NI):
            start_lo(wq_copy(u))
            if u == 1:
                for j in range(S - 1):
                    s_op(j, hop1, start_hi)
        for b in range(LA):
            for j in range(n):
                start_lo(kv_copy(kt_hbm, b, b, j))

        s_ref[...] = jnp.zeros_like(s_ref)
        cp_c.wait()
        cp_x.wait()
        c32 = jnp.broadcast_to(c_v[...].astype(jnp.float32), (8, D))
        sc = (c32 * jax.nn.sigmoid(c32)).astype(jnp.bfloat16)
        x32 = jnp.broadcast_to(x_v[...].astype(jnp.float32), (8, D))
        ln1 = _layernorm(x32)
        cp_ma.wait()
        mod_a = jnp.dot(sc, wma_v[...], preferred_element_type=jnp.float32)
        h = (ln1 * (1.0 + mod_a[:, D:2 * D]) + mod_a[:, 0:D]).astype(jnp.bfloat16)

        row = lax.broadcasted_iota(jnp.int32, (8, BR), 0)
        col = lax.broadcasted_iota(jnp.int32, (8, BR), 1)

        def head_mask(b):
            gcol = col + (b % BPG) * BR
            return jnp.logical_and(gcol >= row * DH, gcol < (row + 1) * DH)

        for u in range(NI):
            wq_copy(u).wait()
            side_traffic(u, u, u)
            if u % NQR == NQR - 1:
                cg = u // NQR
                q = jnp.dot(h, wq_v[:, cg * QC:(cg + 1) * QC], preferred_element_type=jnp.float32)
                for i in range(QC // BR):
                    b = cg * (QC // BR) + i
                    qbd[b] = jnp.where(head_mask(b), q[:, i * BR:(i + 1) * BR], 0.0).astype(jnp.bfloat16)

        for j in range(n):
            kv_step(0, j, 0, 0)

        def k_body(tau, carry):
            b = tau - 1
            slot = b % NB
            qb = qbd[b]
            for j in range(n):
                kv_step(tau, j, 1, NBLK)
                cs = pl.ds(j * CW, CW)
                s_ref[:, cs] += jnp.dot(qb, kv[slot, :, cs], preferred_element_type=jnp.float32)

            @pl.when(b % BPG == BPG - 1)
            def _():
                g = b // BPG
                sg = s_ref[...] * scale
                m = jnp.max(sg, axis=-1, keepdims=True)
                e = jnp.exp(sg - m)
                l = jnp.sum(e, axis=-1, keepdims=True)
                p_ref[g] = e.astype(jnp.bfloat16)
                linv_ref[g] = jnp.broadcast_to(1.0 / l, (8, BR))
                s_ref[...] = jnp.zeros_like(s_ref)
            return carry

        lax.fori_loop(1, NBLK + 1, k_body, 0)

        mod_b = jnp.dot(sc, wmb_v[...], preferred_element_type=jnp.float32)

        def v_block(b, acc, dma):
            slot = (b + NBLK) % NB
            g = b // BPG
            o = jnp.zeros((8, BR), jnp.float32)
            for j in range(n):
                dma(j)
                cs = pl.ds(j * CW, CW)
                o = o + lax.dot_general(p_ref[g, :, cs], kv[slot, :, cs], (((1,), (1,)), ((), ())),
                                        preferred_element_type=jnp.float32)
            o = jnp.where(head_mask(b), o * linv_ref[g], 0.0).astype(jnp.bfloat16)
            r0 = _mult(b * BR, BR)
            return acc + jnp.dot(o, wo_v[pl.ds(r0, BR), :], preferred_element_type=jnp.float32)

        def v_body(tau, acc):
            return v_block(tau - 1 - NBLK, acc, lambda j: kv_step(tau, j, NBLK + 1, 2 * NBLK - 1))

        acc = lax.fori_loop(NBLK + 1, 2 * NBLK, v_body, jnp.zeros((8, D), jnp.float32))

        def last_dma(j):
            if j == n - 1:
                for t in range(NSTEP - TL, NSTEP):
                    trickle_op(t, t, t, wait)
        acc = v_block(NBLK - 1, acc, last_dma)
        attn = jnp.broadcast_to(jnp.sum(acc, axis=0, keepdims=True), (8, D))

        x1 = x32 + mod_b[:, 0:D] * attn
        h2 = (_layernorm(x1) * (1.0 + mod_b[:, 2 * D:3 * D]) + mod_b[:, D:2 * D]).astype(jnp.bfloat16)
        gg = jnp.dot(h2, wg_v[...], preferred_element_type=jnp.float32)
        uu = jnp.dot(h2, wu_v[...], preferred_element_type=jnp.float32)
        hh = (gg * uu).astype(jnp.bfloat16)
        y = jnp.zeros((8, D), jnp.float32)
        r = 0
        for cp, rows in zip(wd_cps, wd_chunks):
            cp.wait()
            y = y + jnp.dot(hh[:, r:r + rows], wd_v[r:r + rows, :], preferred_element_type=jnp.float32)
            r += rows
        out = x1 + mod_b[:, 3 * D:4 * D] * y
        out_ref[...] = out[0:1, :].astype(out_ref.dtype)

    scratch = [
        pltpu.VMEM((1, D), jnp.bfloat16),
        pltpu.VMEM((1, D), jnp.bfloat16),
        pltpu.VMEM((D, 2 * D), jnp.bfloat16),
        pltpu.VMEM((D, 4 * D), jnp.bfloat16),
        pltpu.VMEM((D, ROWS), jnp.bfloat16),
        pltpu.VMEM((ROWS, D), jnp.bfloat16),
        pltpu.VMEM((D, F), jnp.bfloat16),
        pltpu.VMEM((D, F), jnp.bfloat16),
        pltpu.VMEM((F, D), jnp.bfloat16),
        pltpu.VMEM((NB, BR, W), jnp.bfloat16),
        pltpu.VMEM((NBLK, 8, BR), jnp.bfloat16),
        pltpu.VMEM((8, W), jnp.float32),
        pltpu.VMEM((NG, 8, W), jnp.bfloat16),
        pltpu.VMEM((NG, 8, BR), jnp.float32),
        pltpu.SMEM((S, 8, F), jnp.bfloat16),
        pltpu.SemaphoreType.DMA((NSEM,)),
    ]
    return kernel, scratch


@jax.jit
def pallas_adaLN_cond__sliding_block_cached__glu_gated_bilinear__decode_kernel(
    A_x: jax.Array,
    A_k_cache: jax.Array,
    A_v_cache: jax.Array,
    A_wq: jax.Array,
    A_wo: jax.Array,
    B_x: jax.Array,
    B_w_gate: jax.Array,
    B_w_up: jax.Array,
    B_w_down: jax.Array,
    c: jax.Array,
    w_mod: jax.Array,
):
    SK = A_k_cache.shape[2]
    W = min(4096, max(256, SK // 4))
    kt = jnp.swapaxes(A_k_cache, 2, 3).reshape(ROWS, SK)
    vt = jnp.swapaxes(A_v_cache, 2, 3).reshape(ROWS, SK)
    kernel, scratch = make_kernel(SK, W, Rt=64, Wt=2048, every=3, NS=130)
    out = pl.pallas_call(
        kernel,
        in_specs=[pl.BlockSpec(memory_space=pl.ANY)] * 10,
        out_specs=pl.BlockSpec(memory_space=pltpu.VMEM),
        out_shape=jax.ShapeDtypeStruct((1, D), jnp.bfloat16),
        scratch_shapes=scratch,
        compiler_params=pltpu.CompilerParams(vmem_limit_bytes=100 * 1024 * 1024),
    )(A_x.reshape(1, D), c, w_mod, A_wq, kt, vt, A_wo, B_w_gate, B_w_up, B_w_down)
    return out.reshape(1, 1, D)
```

```python
import jax
import jax.numpy as jnp
from jax import lax
import jax.experimental.pallas as pl
import jax.experimental.pallas.tpu as pltpu

D = 640
HQ = 32
DH = 192
ROWS = HQ * DH
F = 1536
GH = 8
GROWS = GH * DH
NG = HQ // GH
EPS = 1e-5
HI, LO = 0, 1


def _layernorm(x):
    m = jnp.mean(x, axis=-1, keepdims=True)
    xc = x - m
    v = jnp.mean(xc * xc, axis=-1, keepdims=True)
    return xc * lax.rsqrt(v + EPS)


def _static(i):
    return isinstance(i, int)


def _mult(i, m):
    return i if _static(i) else pl.multiple_of(i, m)


def _when(cond, fn):
    if isinstance(cond, bool):
        if cond:
            fn()
    else:
        pl.when(cond)(fn)


def _in_range(t, a, b, lo, hi):
    if _static(t):
        return a <= t < b
    if b <= a or b <= lo or a > hi:
        return False
    if a <= lo and hi < b:
        return True
    if a <= lo:
        return t < b
    if hi < b:
        return t >= a
    return jnp.logical_and(t >= a, t < b)


def make_kernel(SK, W, BR=128, Rt=64, Wt=1024, rows_fast=False, LAT=24, NB=8, MR=64,
                every=6, NS=128, S=4, gu_parts=2, nbig=4, wd_chunks=(512, 512, 256, 128, 128),
                scopes=False):
    C0 = SK - W
    scale = DH ** -0.5
    NBLK = ROWS // BR
    BPG = GROWS // BR
    nr, nc = BR // Rt, W // Wt
    n = nr * nc
    CW = W // n
    NI = D // MR
    NSTEP = NI + 2 * NBLK * n
    NP = D // 8
    big_js = [(i * n) // nbig for i in range(nbig)]
    small_js = [j for j in range(n) if j not in big_js]
    nsm = len(small_js)
    q_rows, wo_rows = D // nbig, BR // nbig
    n_mb = 4 * NP
    n_gu = (2 * NP - NS) * gu_parts
    assert sum(wd_chunks) == F
    assert n_mb + n_gu <= (2 * NBLK - 1) * nsm, (n_mb, n_gu, nsm)
    tau_mb = -(-n_mb // nsm) + 1
    assert tau_mb + 4 <= 2 * NBLK
    tau_mb = max(tau_mb, NBLK + 1)
    assert (NS + 1) * every <= NSTEP and NS >= NP
    assert NB * n >= LAT + 2 * n and LAT >= n and NI >= nbig
    o_kv = 0
    o_tr = o_kv + NB * n
    o_s1 = o_tr + 2 * n
    o_s2 = o_s1 + S
    o_in = o_s2 + S
    o_misc = o_in + NI
    o_wd = o_misc + 2
    NSEM = o_wd + len(wd_chunks)

    def kernel(x_hbm, c_hbm, wmod_hbm, wq_hbm, kt_hbm, vt_hbm, wo_hbm, wg_hbm, wu_hbm, wd_hbm,
               out_ref,
               x_v, c_v, wma_v, wmb_v, wq_v, wo_v, wg_v, wu_v, wd_v, kv, qbd, s_ref, p_ref, linv_ref,
               modb_ref, stage, sems):
        cur = [None]

        def mark(name):
            if not scopes:
                return
            if cur[0] is not None:
                cur[0].__exit__(None, None, None)
            cur[0] = jax.named_scope(name) if name else None
            if name:
                cur[0].__enter__()

        start_hi = lambda cp: cp.start(priority=HI)
        start_lo = lambda cp: cp.start(priority=LO)
        wait = lambda cp: cp.wait()

        def kv_copy(src, b, slot, j):
            rj, cj = (j % nr, j // nr) if rows_fast else (j // nc, j % nc)
            r0 = _mult(b * BR + rj * Rt, Rt)
            return pltpu.make_async_copy(
                src.at[pl.ds(r0, Rt), pl.ds(C0 + cj * Wt, Wt)],
                kv.at[slot, pl.ds(rj * Rt, Rt), pl.ds(cj * Wt, Wt)],
                sems.at[o_kv + slot * n + j])

        def init_copy(u):
            return pltpu.make_async_copy(wmod_hbm.at[pl.ds(u * MR, MR), pl.ds(0, 2 * D)],
                                         wma_v.at[pl.ds(u * MR, MR)], sems.at[o_in + u])

        def trickle(item, j, lo, hi, op):
            sem = sems.at[o_tr + (item % 2) * n + j]
            if j in big_js:
                i = big_js.index(j)

                def wq_piece():
                    c0 = _mult(item * BR, BR)
                    op(pltpu.make_async_copy(wq_hbm.at[pl.ds(i * q_rows, q_rows), pl.ds(c0, BR)],
                                             wq_v.at[item % 2, pl.ds(i * q_rows, q_rows)], sem))

                def wo_piece():
                    r0 = _mult((item - NBLK) * BR + i * wo_rows, wo_rows)
                    op(pltpu.make_async_copy(wo_hbm.at[pl.ds(r0, wo_rows)],
                                             wo_v.at[item % 4, pl.ds(i * wo_rows, wo_rows)], sem))

                _when(_in_range(item, 0, NBLK, lo, hi), wq_piece)
                _when(_in_range(item, NBLK, 2 * NBLK, lo, hi), wo_piece)
            else:
                i = small_js.index(j)
                t, tlo, thi = [(v - 1) * nsm + i for v in (item, lo, hi)]

                def mb_piece():
                    r0 = _mult((t // 4) * 8, 8)
                    ch = t % 4
                    op(pltpu.make_async_copy(
                        wmod_hbm.at[pl.ds(r0, 8), pl.ds(_mult(2 * D + ch * D, 128), D)],
                        wmb_v.at[ch, pl.ds(r0, 8)], sem))

                def gu_piece():
                    k = t - n_mb
                    r0 = _mult((k // gu_parts + NS - NP) * 8, 8)
                    cw = F // gu_parts
                    c0 = _mult((k % gu_parts) * cw, 128)
                    op(pltpu.make_async_copy(wu_hbm.at[pl.ds(r0, 8), pl.ds(c0, cw)],
                                             wu_v.at[pl.ds(r0, 8), pl.ds(c0, cw)], sem))

                _when(_in_range(t, 0, n_mb, tlo, thi), mb_piece)
                _when(_in_range(t, n_mb, n_mb + n_gu, tlo, thi), gu_piece)

        def hop1(src, i, j):
            return pltpu.make_async_copy(src.at[pl.ds(_mult(i * 8, 8), 8)], stage.at[j % S],
                                         sems.at[o_s1 + j % S])

        def hop2(dst, i, j):
            return pltpu.make_async_copy(stage.at[j % S], dst.at[pl.ds(_mult(i * 8, 8), 8)],
                                         sems.at[o_s2 + j % S])

        def s_op(j, lo, hi, hop, op):
            a, b = (wg_hbm, wu_hbm) if hop is hop1 else (wg_v, wu_v)
            _when(_in_range(j, 0, NP, lo, hi), lambda: op(hop(a, j, j)))
            _when(_in_range(j, NP, NS, lo, hi), lambda: op(hop(b, j - NP, j)))

        def smem_tick(j, lo, hi):
            s_op(j, lo, hi, hop1, wait)
            s_op(j, lo, hi, hop2, start_hi)
            s_op(j - 1, lo - 1, hi - 1, hop2, wait)
            s_op(j + S - 1, lo + S - 1, hi + S - 1, hop1, start_hi)

        def smem_step(u, lo, hi, stride):
            if not any(v % every == every - 1 for v in range(lo, hi + 1, stride)):
                return
            always = all(v % every == every - 1 for v in range(lo, hi + 1, stride))
            _when(True if always else u % every == every - 1,
                  lambda: smem_tick(u // every, lo // every, hi // every))

        wd_cps = []
        r = 0
        for i, rows in enumerate(wd_chunks):
            wd_cps.append(pltpu.make_async_copy(wd_hbm.at[pl.ds(r, rows)], wd_v.at[pl.ds(r, rows)],
                                                sems.at[o_wd + i]))
            r += rows

        def issue_kv(b, j, lo, hi):
            slot = b % NB
            _when(_in_range(b, 0, NBLK, lo, hi), lambda: start_lo(kv_copy(kt_hbm, b, slot, j)))
            _when(_in_range(b, NBLK, 2 * NBLK, lo, hi),
                  lambda: start_lo(kv_copy(vt_hbm, b - NBLK, slot, j)))
            if j == n - 1:
                def tail():
                    for cp in wd_cps:
                        start_lo(cp)
                _when(_in_range(b, 2 * NBLK - 1, 2 * NBLK, lo, hi), tail)

        def issue_lo(u):
            if u < NI:
                start_lo(init_copy(u))
            else:
                b, j = (u - NI) // n, (u - NI) % n
                issue_kv(b, j, b, b)

        def kv_step(tau, j, lo, hi):
            kv_copy(kt_hbm, 0, tau % NB, j).wait()
            trickle(tau + 1, j, lo + 1, hi + 1, start_hi)
            db, jn = (j + LAT) // n, (j + LAT) % n
            issue_kv(tau + db, jn, lo + db, hi + db)
            trickle(tau, j, lo, hi, wait)
            smem_step(NI + tau * n + j, NI + lo * n + j, NI + hi * n + j, n)

        cp_c = pltpu.make_async_copy(c_hbm, c_v, sems.at[o_misc])
        cp_x = pltpu.make_async_copy(x_hbm, x_v, sems.at[o_misc + 1])

        mark('p0_issue')
        issue_lo(0)
        start_hi(cp_c)
        start_hi(cp_x)
        for u in range(1, LAT):
            issue_lo(u)
            if u == 3:
                for j in range(S - 1):
                    s_op(j, j, j, hop1, start_hi)

        mark('p1_init')
        s_ref[...] = jnp.zeros_like(s_ref)
        cp_c.wait()
        cp_x.wait()
        c32 = jnp.broadcast_to(c_v[...].astype(jnp.float32), (8, D))
        sc = (c32 * jax.nn.sigmoid(c32)).astype(jnp.bfloat16)
        x32 = jnp.broadcast_to(x_v[...].astype(jnp.float32), (8, D))
        ln1 = _layernorm(x32)

        row = lax.broadcasted_iota(jnp.int32, (8, BR), 0)
        col = lax.broadcasted_iota(jnp.int32, (8, BR), 1)

        def head_mask(b):
            gcol = col + (b % BPG) * BR
            return jnp.logical_and(gcol >= row * DH, gcol < (row + 1) * DH)

        init_big = [(i * NI) // nbig for i in range(nbig)]
        for u in range(NI):
            init_copy(u).wait()
            if u in init_big:
                trickle(0, big_js[init_big.index(u)], 0, 0, start_hi)
            issue_lo(u + LAT)
            smem_step(u, u, u, 1)
        mod_a = jnp.dot(sc, wma_v[...], preferred_element_type=jnp.float32)
        h = (ln1 * (1.0 + mod_a[:, D:2 * D]) + mod_a[:, 0:D]).astype(jnp.bfloat16)

        def q_block(b):
            q = jnp.dot(h, wq_v[b % 2], preferred_element_type=jnp.float32)
            qbd[...] = jnp.where(head_mask(b), q, 0.0).astype(jnp.bfloat16)

        mark('p3_tau0')
        for j in range(n):
            kv_step(0, j, 0, 0)
        q_block(0)

        def k_body(tau, carry):
            b = tau - 1
            slot = b % NB
            qb = qbd[...]
            for j in range(n):
                kv_step(tau, j, 1, NBLK)
                cs = pl.ds(j * CW, CW)
                s_ref[:, cs] += jnp.dot(qb, kv[slot, :, cs], preferred_element_type=jnp.float32)

            @pl.when(tau < NBLK)
            def _():
                q_block(tau)

            @pl.when(b % BPG == BPG - 1)
            def _():
                g = b // BPG
                sg = s_ref[...] * scale
                m = jnp.max(sg, axis=-1, keepdims=True)
                e = jnp.exp(sg - m)
                l = jnp.sum(e, axis=-1, keepdims=True)
                p_ref[g] = e.astype(jnp.bfloat16)
                linv_ref[g] = jnp.broadcast_to(1.0 / l, (8, BR))
                s_ref[...] = jnp.zeros_like(s_ref)
            return carry

        mark('p4_kloop')
        lax.fori_loop(1, NBLK + 1, k_body, 0)

        def v_block(b, acc, dma):
            slot = (b + NBLK) % NB
            g = b // BPG
            o = jnp.zeros((8, BR), jnp.float32)
            for j in range(n):
                dma(j)
                cs = pl.ds(j * CW, CW)
                o = o + lax.dot_general(p_ref[g, :, cs], kv[slot, :, cs], (((1,), (1,)), ((), ())),
                                        preferred_element_type=jnp.float32)
            o = jnp.where(head_mask(b), o * linv_ref[g], 0.0).astype(jnp.bfloat16)
            return acc + jnp.dot(o, wo_v[(b + NBLK) % 4], preferred_element_type=jnp.float32)

        def v_body(tau, acc):
            acc = v_block(tau - 1 - NBLK, acc, lambda j: kv_step(tau, j, NBLK + 1, 2 * NBLK - 1))

            @pl.when(jnp.logical_and(tau >= tau_mb, tau < tau_mb + 4))
            def _():
                ch = tau - tau_mb
                modb_ref[ch] = jnp.dot(sc, wmb_v[ch], preferred_element_type=jnp.float32)
            return acc

        mark('p6_vloop')
        acc = lax.fori_loop(NBLK + 1, 2 * NBLK, v_body, jnp.zeros((8, D), jnp.float32))

        mark('p7_lastv')
        acc = v_block(NBLK - 1, acc, lambda j: None)
        mark('p8_ln_gu')
        attn = jnp.broadcast_to(jnp.sum(acc, axis=0, keepdims=True), (8, D))

        x1 = x32 + modb_ref[0] * attn
        h2 = (_layernorm(x1) * (1.0 + modb_ref[2]) + modb_ref[1]).astype(jnp.bfloat16)
        gg = jnp.dot(h2, wg_v[...], preferred_element_type=jnp.float32)
        uu = jnp.dot(h2, wu_v[...], preferred_element_type=jnp.float32)
        hh = (gg * uu).astype(jnp.bfloat16)
        mark('p9_wd')
        y = jnp.zeros((8, D), jnp.float32)
        r = 0
        for cp, rows in zip(wd_cps, wd_chunks):
            cp.wait()
            y = y + jnp.dot(hh[:, r:r + rows], wd_v[r:r + rows, :], preferred_element_type=jnp.float32)
            r += rows
        out = x1 + modb_ref[3] * y
        out_ref[...] = out[0:1, :].astype(out_ref.dtype)
        mark(None)

    scratch = [
        pltpu.VMEM((1, D), jnp.bfloat16),
        pltpu.VMEM((1, D), jnp.bfloat16),
        pltpu.VMEM((D, 2 * D), jnp.bfloat16),
        pltpu.VMEM((4, D, D), jnp.bfloat16),
        pltpu.VMEM((2, D, BR), jnp.bfloat16),
        pltpu.VMEM((4, BR, D), jnp.bfloat16),
        pltpu.VMEM((D, F), jnp.bfloat16),
        pltpu.VMEM((D, F), jnp.bfloat16),
        pltpu.VMEM((F, D), jnp.bfloat16),
        pltpu.VMEM((NB, BR, W), jnp.bfloat16),
        pltpu.VMEM((8, BR), jnp.bfloat16),
        pltpu.VMEM((8, W), jnp.float32),
        pltpu.VMEM((NG, 8, W), jnp.bfloat16),
        pltpu.VMEM((NG, 8, BR), jnp.float32),
        pltpu.VMEM((4, 8, D), jnp.float32),
        pltpu.SMEM((S, 8, F), jnp.bfloat16),
        pltpu.SemaphoreType.DMA((NSEM,)),
    ]
    return kernel, scratch


@jax.jit
def pallas_adaLN_cond__sliding_block_cached__glu_gated_bilinear__decode_kernel(
    A_x: jax.Array,
    A_k_cache: jax.Array,
    A_v_cache: jax.Array,
    A_wq: jax.Array,
    A_wo: jax.Array,
    B_x: jax.Array,
    B_w_gate: jax.Array,
    B_w_up: jax.Array,
    B_w_down: jax.Array,
    c: jax.Array,
    w_mod: jax.Array,
):
    SK = A_k_cache.shape[2]
    W = min(4096, max(256, SK // 4))
    kt = jnp.swapaxes(A_k_cache, 2, 3).reshape(ROWS, SK)
    vt = jnp.swapaxes(A_v_cache, 2, 3).reshape(ROWS, SK)
    kernel, scratch = make_kernel(SK, W, gu_parts=1)
    out = pl.pallas_call(
        kernel,
        in_specs=[pl.BlockSpec(memory_space=pl.ANY)] * 10,
        out_specs=pl.BlockSpec(memory_space=pltpu.VMEM),
        out_shape=jax.ShapeDtypeStruct((1, D), jnp.bfloat16),
        scratch_shapes=scratch,
        compiler_params=pltpu.CompilerParams(vmem_limit_bytes=64 * 1024 * 1024,
                                             disable_semaphore_checks=True,
                                             disable_bounds_checks=True),
    )(A_x.reshape(1, D), c, w_mod, A_wq, kt, vt, A_wo, B_w_gate, B_w_up, B_w_down)
    return out.reshape(1, 1, D)
```

```python
import jax
import jax.numpy as jnp
from jax import lax
import jax.experimental.pallas as pl
import jax.experimental.pallas.tpu as pltpu

D = 640
HQ = 32
DH = 192
ROWS = HQ * DH
F = 1536
GH = 8
GROWS = GH * DH
NG = HQ // GH
EPS = 1e-5
HI, LO = 0, 1


def _layernorm(x):
    m = jnp.mean(x, axis=-1, keepdims=True)
    xc = x - m
    v = jnp.mean(xc * xc, axis=-1, keepdims=True)
    return xc * lax.rsqrt(v + EPS)


def _static(i):
    return isinstance(i, int)


def _mult(i, m):
    return i if _static(i) else pl.multiple_of(i, m)


def _when(cond, fn):
    if isinstance(cond, bool):
        if cond:
            fn()
    else:
        pl.when(cond)(fn)


def _in_range(t, a, b, lo, hi):
    if _static(t):
        return a <= t < b
    if b <= a or b <= lo or a > hi:
        return False
    if a <= lo and hi < b:
        return True
    if a <= lo:
        return t < b
    if hi < b:
        return t >= a
    return jnp.logical_and(t >= a, t < b)


def make_kernel(SK, W, BR=128, Rt=64, Wt=1024, rows_fast=True, coff=0, tiles=None, LAT=24, NB=8, MR=64,
                every=6, NS=128, S=4, gu_parts=1, nbig=4, wd_chunks=(512, 512, 256, 128, 128),
                scopes=False, gu_tail=0):
    C0 = SK - W
    scale = DH ** -0.5
    NBLK = ROWS // BR
    BPG = GROWS // BR
    nr, nc = BR // Rt, W // Wt
    n = nr * nc
    CW = W // n
    NI = D // MR
    NSTEP = NI + 2 * NBLK * n
    NP = D // 8
    big_js = [(i * n) // nbig for i in range(nbig)]
    small_js = [j for j in range(n) if j not in big_js]
    nsm = len(small_js)
    q_rows, wo_rows = D // nbig, BR // nbig
    n_mb = 4 * NP
    n_gu = (2 * NP - NS - gu_tail) * gu_parts
    assert sum(wd_chunks) == F
    assert n_mb + n_gu <= (2 * NBLK - 1) * nsm, (n_mb, n_gu, nsm)
    tau_mb = -(-n_mb // nsm) + 1
    assert tau_mb + 4 <= 2 * NBLK
    tau_mb = max(tau_mb, NBLK + 1)
    assert (NS + 1) * every <= NSTEP and NS >= NP
    assert NB * n >= LAT + 2 * n and LAT >= n and NI >= nbig
    if tiles is None:
        tiles = []
        for j in range(n):
            rj, cj = (j % nr, j // nr) if rows_fast else (j // nc, j % nc)
            c0 = cj * Wt + coff
            if c0 + Wt <= W:
                tiles.append([(rj * Rt, Rt, c0, Wt)])
            else:
                tiles.append([(rj * Rt, Rt, c0, W - c0), (rj * Rt, Rt, 0, coff)])
    assert len(tiles) == n
    cover = sorted((r, c) for st in tiles for (r0, rn, c0, cn) in st
                   for r in range(r0, r0 + rn, 8) for c in range(c0, c0 + cn, 128))
    assert cover == [(r, c) for r in range(0, BR, 8) for c in range(0, W, 128)]
    sem_of = {}
    for j in range(n):
        for k in range(len(tiles[j])):
            sem_of[(j, k)] = len(sem_of)
    nks = len(sem_of)
    o_kv = 0
    o_tr = o_kv + NB * nks
    o_s1 = o_tr + 2 * n
    o_s2 = o_s1 + S
    o_in = o_s2 + S
    o_misc = o_in + NI
    o_wd = o_misc + 2
    NSEM = o_wd + len(wd_chunks) + 1

    def kernel(x_hbm, c_hbm, wmod_hbm, wq_hbm, kt_hbm, vt_hbm, wo_hbm, wg_hbm, wu_hbm, wd_hbm,
               out_ref,
               x_v, c_v, wma_v, wmb_v, wq_v, wo_v, wg_v, wu_v, wd_v, kv, qbd, s_ref, p_ref, linv_ref,
               modb_ref, stage, sems):
        cur = [None]

        def mark(name):
            if not scopes:
                return
            if cur[0] is not None:
                cur[0].__exit__(None, None, None)
            cur[0] = jax.named_scope(name) if name else None
            if name:
                cur[0].__enter__()

        start_hi = lambda cp: cp.start(priority=HI)
        start_lo = lambda cp: cp.start(priority=LO)
        wait = lambda cp: cp.wait()

        def kv_op(src, b, slot, j, op):
            for k, (rt, rn, ct, cn) in enumerate(tiles[j]):
                op(pltpu.make_async_copy(
                    src.at[pl.ds(_mult(b * BR + rt, 8), rn), pl.ds(C0 + ct, cn)],
                    kv.at[slot, pl.ds(rt, rn), pl.ds(ct, cn)],
                    sems.at[o_kv + slot * nks + sem_of[(j, k)]]))

        def init_copy(u):
            return pltpu.make_async_copy(wmod_hbm.at[pl.ds(u * MR, MR), pl.ds(0, 2 * D)],
                                         wma_v.at[pl.ds(u * MR, MR)], sems.at[o_in + u])

        def trickle(item, j, lo, hi, op):
            sem = sems.at[o_tr + (item % 2) * n + j]
            if j in big_js:
                i = big_js.index(j)

                def wq_piece():
                    c0 = _mult(item * BR, BR)
                    op(pltpu.make_async_copy(wq_hbm.at[pl.ds(i * q_rows, q_rows), pl.ds(c0, BR)],
                                             wq_v.at[item % 2, pl.ds(i * q_rows, q_rows)], sem))

                def wo_piece():
                    r0 = _mult((item - NBLK) * BR + i * wo_rows, wo_rows)
                    op(pltpu.make_async_copy(wo_hbm.at[pl.ds(r0, wo_rows)],
                                             wo_v.at[item % 4, pl.ds(i * wo_rows, wo_rows)], sem))

                _when(_in_range(item, 0, NBLK, lo, hi), wq_piece)
                _when(_in_range(item, NBLK, 2 * NBLK, lo, hi), wo_piece)
            else:
                i = small_js.index(j)
                t, tlo, thi = [(v - 1) * nsm + i for v in (item, lo, hi)]

                def mb_piece():
                    r0 = _mult((t // 4) * 8, 8)
                    ch = t % 4
                    op(pltpu.make_async_copy(
                        wmod_hbm.at[pl.ds(r0, 8), pl.ds(_mult(2 * D + ch * D, 128), D)],
                        wmb_v.at[ch, pl.ds(r0, 8)], sem))

                def gu_piece():
                    k = t - n_mb
                    r0 = _mult((k // gu_parts + NS - NP) * 8, 8)
                    cw = F // gu_parts
                    c0 = _mult((k % gu_parts) * cw, 128)
                    op(pltpu.make_async_copy(wu_hbm.at[pl.ds(r0, 8), pl.ds(c0, cw)],
                                             wu_v.at[pl.ds(r0, 8), pl.ds(c0, cw)], sem))

                _when(_in_range(t, 0, n_mb, tlo, thi), mb_piece)
                _when(_in_range(t, n_mb, n_mb + n_gu, tlo, thi), gu_piece)

        def hop1(src, i, j):
            return pltpu.make_async_copy(src.at[pl.ds(_mult(i * 8, 8), 8)], stage.at[j % S],
                                         sems.at[o_s1 + j % S])

        def hop2(dst, i, j):
            return pltpu.make_async_copy(stage.at[j % S], dst.at[pl.ds(_mult(i * 8, 8), 8)],
                                         sems.at[o_s2 + j % S])

        def s_op(j, lo, hi, hop, op):
            a, b = (wg_hbm, wu_hbm) if hop is hop1 else (wg_v, wu_v)
            _when(_in_range(j, 0, NP, lo, hi), lambda: op(hop(a, j, j)))
            _when(_in_range(j, NP, NS, lo, hi), lambda: op(hop(b, j - NP, j)))

        def smem_tick(j, lo, hi):
            s_op(j, lo, hi, hop1, wait)
            s_op(j, lo, hi, hop2, start_hi)
            s_op(j - 1, lo - 1, hi - 1, hop2, wait)
            s_op(j + S - 1, lo + S - 1, hi + S - 1, hop1, start_hi)

        def smem_step(u, lo, hi, stride):
            if not any(v % every == every - 1 for v in range(lo, hi + 1, stride)):
                return
            always = all(v % every == every - 1 for v in range(lo, hi + 1, stride))
            _when(True if always else u % every == every - 1,
                  lambda: smem_tick(u // every, lo // every, hi // every))

        wd_cps = []
        r = 0
        for i, rows in enumerate(wd_chunks):
            wd_cps.append(pltpu.make_async_copy(wd_hbm.at[pl.ds(r, rows)], wd_v.at[pl.ds(r, rows)],
                                                sems.at[o_wd + i]))
            r += rows

        def gu_tail_copy():
            r0 = D - 8 * gu_tail
            return pltpu.make_async_copy(wu_hbm.at[pl.ds(r0, 8 * gu_tail)], wu_v.at[pl.ds(r0, 8 * gu_tail)],
                                         sems.at[NSEM - 1])

        def issue_kv(b, j, lo, hi):
            slot = b % NB
            _when(_in_range(b, 0, NBLK, lo, hi), lambda: kv_op(kt_hbm, b, slot, j, start_lo))
            _when(_in_range(b, NBLK, 2 * NBLK, lo, hi),
                  lambda: kv_op(vt_hbm, b - NBLK, slot, j, start_lo))
            if j == n - 1:
                def tail():
                    if gu_tail:
                        start_lo(gu_tail_copy())
                    for cp in wd_cps:
                        start_lo(cp)
                _when(_in_range(b, 2 * NBLK - 1, 2 * NBLK, lo, hi), tail)

        def issue_lo(u):
            if u < NI:
                start_lo(init_copy(u))
            else:
                b, j = (u - NI) // n, (u - NI) % n
                issue_kv(b, j, b, b)

        def kv_step(tau, j, lo, hi):
            kv_op(kt_hbm, 0, tau % NB, j, wait)
            trickle(tau + 1, j, lo + 1, hi + 1, start_hi)
            db, jn = (j + LAT) // n, (j + LAT) % n
            issue_kv(tau + db, jn, lo + db, hi + db)
            trickle(tau, j, lo, hi, wait)
            smem_step(NI + tau * n + j, NI + lo * n + j, NI + hi * n + j, n)

        cp_c = pltpu.make_async_copy(c_hbm, c_v, sems.at[o_misc])
        cp_x = pltpu.make_async_copy(x_hbm, x_v, sems.at[o_misc + 1])

        mark('p0_issue')
        issue_lo(0)
        start_hi(cp_c)
        start_hi(cp_x)
        for u in range(1, LAT):
            issue_lo(u)
            if u == 3:
                for j in range(S - 1):
                    s_op(j, j, j, hop1, start_hi)

        mark('p1_init')
        s_ref[...] = jnp.zeros_like(s_ref)
        cp_c.wait()
        cp_x.wait()
        c32 = jnp.broadcast_to(c_v[...].astype(jnp.float32), (8, D))
        sc = (c32 * jax.nn.sigmoid(c32)).astype(jnp.bfloat16)
        x32 = jnp.broadcast_to(x_v[...].astype(jnp.float32), (8, D))
        ln1 = _layernorm(x32)

        row = lax.broadcasted_iota(jnp.int32, (8, BR), 0)
        col = lax.broadcasted_iota(jnp.int32, (8, BR), 1)

        def head_mask(b):
            gcol = col + (b % BPG) * BR
            return jnp.logical_and(gcol >= row * DH, gcol < (row + 1) * DH)

        init_big = [(i * NI) // nbig for i in range(nbig)]
        for u in range(NI):
            init_copy(u).wait()
            if u in init_big:
                trickle(0, big_js[init_big.index(u)], 0, 0, start_hi)
            issue_lo(u + LAT)
            smem_step(u, u, u, 1)
        mod_a = jnp.dot(sc, wma_v[...], preferred_element_type=jnp.float32)
        h = (ln1 * (1.0 + mod_a[:, D:2 * D]) + mod_a[:, 0:D]).astype(jnp.bfloat16)

        def q_block(b):
            q = jnp.dot(h, wq_v[b % 2], preferred_element_type=jnp.float32)
            qbd[...] = jnp.where(head_mask(b), q, 0.0).astype(jnp.bfloat16)

        mark('p3_tau0')
        for j in range(n):
            kv_step(0, j, 0, 0)
        q_block(0)

        def k_body(tau, carry):
            b = tau - 1
            slot = b % NB
            qb = qbd[...]
            for j in range(n):
                kv_step(tau, j, 1, NBLK)
                cs = pl.ds(j * CW, CW)
                s_ref[:, cs] += jnp.dot(qb, kv[slot, :, cs], preferred_element_type=jnp.float32)

            @pl.when(tau < NBLK)
            def _():
                q_block(tau)

            @pl.when(b % BPG == BPG - 1)
            def _():
                g = b // BPG
                sg = s_ref[...] * scale
                m = jnp.max(sg, axis=-1, keepdims=True)
                e = jnp.exp(sg - m)
                l = jnp.sum(e, axis=-1, keepdims=True)
                p_ref[g] = e.astype(jnp.bfloat16)
                linv_ref[g] = jnp.broadcast_to(1.0 / l, (8, BR))
                s_ref[...] = jnp.zeros_like(s_ref)
            return carry

        mark('p4_kloop')
        lax.fori_loop(1, NBLK + 1, k_body, 0)

        def v_block(b, acc, dma):
            slot = (b + NBLK) % NB
            g = b // BPG
            o = jnp.zeros((8, BR), jnp.float32)
            for j in range(n):
                dma(j)
                cs = pl.ds(j * CW, CW)
                o = o + lax.dot_general(p_ref[g, :, cs], kv[slot, :, cs], (((1,), (1,)), ((), ())),
                                        preferred_element_type=jnp.float32)
            o = jnp.where(head_mask(b), o * linv_ref[g], 0.0).astype(jnp.bfloat16)
            return acc + jnp.dot(o, wo_v[(b + NBLK) % 4], preferred_element_type=jnp.float32)

        def v_body(tau, acc):
            acc = v_block(tau - 1 - NBLK, acc, lambda j: kv_step(tau, j, NBLK + 1, 2 * NBLK - 1))

            @pl.when(jnp.logical_and(tau >= tau_mb, tau < tau_mb + 4))
            def _():
                ch = tau - tau_mb
                modb_ref[ch] = jnp.dot(sc, wmb_v[ch], preferred_element_type=jnp.float32)
            return acc

        mark('p6_vloop')
        acc = lax.fori_loop(NBLK + 1, 2 * NBLK, v_body, jnp.zeros((8, D), jnp.float32))

        mark('p7_lastv')
        acc = v_block(NBLK - 1, acc, lambda j: None)
        mark('p8_ln_gu')
        attn = jnp.broadcast_to(jnp.sum(acc, axis=0, keepdims=True), (8, D))

        x1 = x32 + modb_ref[0] * attn
        h2 = (_layernorm(x1) * (1.0 + modb_ref[2]) + modb_ref[1]).astype(jnp.bfloat16)
        gg = jnp.dot(h2, wg_v[...], preferred_element_type=jnp.float32)
        if gu_tail:
            gu_tail_copy().wait()
        uu = jnp.dot(h2, wu_v[...], preferred_element_type=jnp.float32)
        hh = (gg * uu).astype(jnp.bfloat16)
        mark('p9_wd')
        y = jnp.zeros((8, D), jnp.float32)
        r = 0
        for i, (cp, rows) in enumerate(zip(wd_cps, wd_chunks)):
            mark('p9_w%d' % i)
            cp.wait()
            mark('p9_x%d' % i)
            y = y + jnp.dot(hh[:, r:r + rows], wd_v[r:r + rows, :], preferred_element_type=jnp.float32)
            r += rows
        out = x1 + modb_ref[3] * y
        out_ref[...] = out[0:1, :].astype(out_ref.dtype)
        mark(None)

    scratch = [
        pltpu.VMEM((1, D), jnp.bfloat16),
        pltpu.VMEM((1, D), jnp.bfloat16),
        pltpu.VMEM((D, 2 * D), jnp.bfloat16),
        pltpu.VMEM((4, D, D), jnp.bfloat16),
        pltpu.VMEM((2, D, BR), jnp.bfloat16),
        pltpu.VMEM((4, BR, D), jnp.bfloat16),
        pltpu.VMEM((D, F), jnp.bfloat16),
        pltpu.VMEM((D, F), jnp.bfloat16),
        pltpu.VMEM((F, D), jnp.bfloat16),
        pltpu.VMEM((NB, BR, W), jnp.bfloat16),
        pltpu.VMEM((8, BR), jnp.bfloat16),
        pltpu.VMEM((8, W), jnp.float32),
        pltpu.VMEM((NG, 8, W), jnp.bfloat16),
        pltpu.VMEM((NG, 8, BR), jnp.float32),
        pltpu.VMEM((4, 8, D), jnp.float32),
        pltpu.SMEM((S, 8, F), jnp.bfloat16),
        pltpu.SemaphoreType.DMA((NSEM,)),
    ]
    return kernel, scratch


@jax.jit
def pallas_adaLN_cond__sliding_block_cached__glu_gated_bilinear__decode_kernel(
    A_x: jax.Array,
    A_k_cache: jax.Array,
    A_v_cache: jax.Array,
    A_wq: jax.Array,
    A_wo: jax.Array,
    B_x: jax.Array,
    B_w_gate: jax.Array,
    B_w_up: jax.Array,
    B_w_down: jax.Array,
    c: jax.Array,
    w_mod: jax.Array,
):
    SK = A_k_cache.shape[2]
    W = min(4096, max(256, SK // 4))
    kt = jnp.swapaxes(A_k_cache, 2, 3).reshape(ROWS, SK)
    vt = jnp.swapaxes(A_v_cache, 2, 3).reshape(ROWS, SK)
    kernel, scratch = make_kernel(SK, W, tiles=[[(0, 64, 256, 1024)], [(64, 64, 256, 1024)], [(0, 64, 1280, 1024)], [(64, 64, 1280, 1024)], [(0, 64, 2304, 1024)], [(64, 64, 2304, 1024)], [(0, 128, 3328, 512)], [(0, 128, 3840, 256), (0, 128, 0, 256)]])
    out = pl.pallas_call(
        kernel,
        in_specs=[pl.BlockSpec(memory_space=pl.ANY)] * 10,
        out_specs=pl.BlockSpec(memory_space=pltpu.VMEM),
        out_shape=jax.ShapeDtypeStruct((1, D), jnp.bfloat16),
        scratch_shapes=scratch,
        compiler_params=pltpu.CompilerParams(vmem_limit_bytes=64 * 1024 * 1024,
                                             disable_semaphore_checks=True,
                                             disable_bounds_checks=True),
    )(A_x.reshape(1, D), c, w_mod, A_wq, kt, vt, A_wo, B_w_gate, B_w_up, B_w_down)
    return out.reshape(1, 1, D)
```

```python
import jax
import jax.numpy as jnp
from jax import lax
import jax.experimental.pallas as pl
import jax.experimental.pallas.tpu as pltpu

D = 640
HQ = 32
DH = 192
ROWS = HQ * DH
F = 1536
GH = 8
GROWS = GH * DH
NG = HQ // GH
BR = 128
NBLK = ROWS // BR
BPG = GROWS // BR
NP = D // 8
EPS = 1e-5
HI, LO = 0, 1


def _layernorm(x):
    m = jnp.mean(x, axis=-1, keepdims=True)
    xc = x - m
    v = jnp.mean(xc * xc, axis=-1, keepdims=True)
    return xc * lax.rsqrt(v + EPS)


def _static(i):
    return isinstance(i, int)


def _mult(i, m):
    return i if _static(i) else pl.multiple_of(i, m)


def _mod2(i, m):
    return i % m if _static(i) else jnp.bitwise_and(i, m - 1)


def _when(cond, fn):
    if isinstance(cond, bool):
        if cond:
            fn()
    else:
        pl.when(cond)(fn)


def _in_range(t, a, b, lo, hi):
    if _static(t):
        return a <= t < b
    if b <= a or b <= lo or a > hi:
        return False
    if a <= lo and hi < b:
        return True
    if a <= lo:
        return t < b
    if hi < b:
        return t >= a
    return jnp.logical_and(t >= a, t < b)


def make_kernel(SK, W, tiles, plan, LAT=24, NB=8, MR=64, S=4, sched=((1, 7), (5,), (3,)),
                wd_chunks=(512, 512, 256, 128, 128), gu_tail=0, scopes=False):
    C0 = SK - W
    scale = DH ** -0.5
    n = len(tiles)
    CW = W // n
    NI = D // MR
    cover = sorted((r, c) for st in tiles for (r0, rn, c0, cn) in st
                   for r in range(r0, r0 + rn, 8) for c in range(c0, c0 + cn, 128))
    assert cover == [(r, c) for r in range(0, BR, 8) for c in range(0, W, 128)]
    slots = []
    for j, phases in enumerate(plan):
        for ph, kinds in enumerate(phases):
            for k in kinds:
                slots.append((j, ph, k, sum(1 for s in slots if s[2] == k)))
    nsl = len(slots)
    nbig = sum(1 for s in slots if s[2] == 'b')
    nsm = nsl - nbig
    assert nsm == 4
    q_rows, wo_rows = D // nbig, BR // nbig
    n_init_ticks = 1
    sper = len(sched)

    def ticks_before(tau):
        return n_init_ticks + sum(len(sched[t % sper]) for t in range(tau))
    NS = ticks_before(2 * NBLK) - 1
    assert NP <= NS <= 2 * NP
    n_gu = 2 * NP - NS - gu_tail
    wd_pre = F - sum(wd_chunks)
    assert wd_pre in (0, BR)
    assert n_gu <= (2 * NBLK - 1 - NP) * nsm
    tau_mb = NP + 1
    assert NB * n >= LAT + 2 * n and LAT >= n
    sem_of = {}
    for j in range(n):
        for k in range(len(tiles[j])):
            sem_of[(j, k)] = len(sem_of)
    nks = len(sem_of)
    o_kv = 0
    o_tr = o_kv + NB * nks
    o_s1 = o_tr + 2 * nsl
    o_s2 = o_s1 + S
    o_in = o_s2 + S
    o_misc = o_in + NI
    o_wd = o_misc + 2
    NSEM = o_wd + len(wd_chunks) + 1

    def kernel(x_hbm, c_hbm, wmod_hbm, wq_hbm, kt_hbm, vt_hbm, wo_hbm, wg_hbm, wu_hbm, wd_hbm,
               out_ref,
               x_v, c_v, wma_v, wmb_v, wq_v, wo_v, wg_v, wu_v, wd_v, kv, qbd, s_ref, p_ref, linv_ref,
               modb_ref, stage, sems):
        cur = [None]

        def mark(name):
            if not scopes:
                return
            if cur[0] is not None:
                cur[0].__exit__(None, None, None)
            cur[0] = jax.named_scope(name) if name else None
            if name:
                cur[0].__enter__()

        start_hi = lambda cp: cp.start(priority=HI)
        start_lo = lambda cp: cp.start(priority=LO)
        wait = lambda cp: cp.wait()

        def kv_op(src, b, slot, j, op):
            for k, (rt, rn, ct, cn) in enumerate(tiles[j]):
                op(pltpu.make_async_copy(
                    src.at[pl.ds(_mult(b * BR + rt, 8), rn), pl.ds(C0 + ct, cn)],
                    kv.at[slot, pl.ds(rt, rn), pl.ds(ct, cn)],
                    sems.at[o_kv + slot * nks + sem_of[(j, k)]]))

        def init_copy(u):
            return pltpu.make_async_copy(wmod_hbm.at[pl.ds(u * MR, MR), pl.ds(0, 2 * D)],
                                         wma_v.at[pl.ds(u * MR, MR)], sems.at[o_in + u])

        def trickle(item, si, lo, hi, op):
            _, _, kind, i = slots[si]
            sem = sems.at[o_tr + _mod2(item, 2) * nsl + si]
            if kind == 'b':
                def wq_piece():
                    op(pltpu.make_async_copy(
                        wq_hbm.at[pl.ds(i * q_rows, q_rows), pl.ds(_mult(item * BR, BR), BR)],
                        wq_v.at[_mod2(item, 2), pl.ds(i * q_rows, q_rows)], sem))

                def wo_piece():
                    r0 = _mult((item - NBLK) * BR + i * wo_rows, wo_rows)
                    op(pltpu.make_async_copy(wo_hbm.at[pl.ds(r0, wo_rows)],
                                             wo_v.at[_mod2(item, 4), pl.ds(i * wo_rows, wo_rows)], sem))

                _when(_in_range(item, 0, NBLK, lo, hi), wq_piece)
                _when(_in_range(item, NBLK, 2 * NBLK, lo, hi), wo_piece)
                if wd_pre:
                    rs = pl.ds(i * wo_rows, wo_rows)
                    _when(_in_range(item, 2 * NBLK, 2 * NBLK + 1, lo, hi),
                          lambda: op(pltpu.make_async_copy(wd_hbm.at[rs], wd_v.at[rs], sem)))
            else:
                def mb_piece():
                    r0 = _mult((item - 1) * 8, 8)
                    op(pltpu.make_async_copy(wmod_hbm.at[pl.ds(r0, 8), pl.ds((2 + i) * D, D)],
                                             wmb_v.at[i, pl.ds(r0, 8)], sem))

                def gu_piece():
                    r0 = _mult(((item - 1 - NP) * nsm + i + NS - NP) * 8, 8)
                    op(pltpu.make_async_copy(wu_hbm.at[pl.ds(r0, 8)], wu_v.at[pl.ds(r0, 8)], sem))

                _when(_in_range(item, 1, NP + 1, lo, hi), mb_piece)
                _when(_in_range(item, NP + 1, NP + 1 + (n_gu - i + nsm - 1) // nsm, lo, hi), gu_piece)

        def hop1(src, i, j):
            return pltpu.make_async_copy(src.at[pl.ds(_mult(i * 8, 8), 8)], stage.at[_mod2(j, S)],
                                         sems.at[o_s1 + _mod2(j, S)])

        def hop2(dst, i, j):
            return pltpu.make_async_copy(stage.at[_mod2(j, S)], dst.at[pl.ds(_mult(i * 8, 8), 8)],
                                         sems.at[o_s2 + _mod2(j, S)])

        def s_op(j, lo, hi, hop, op):
            a, b = (wg_hbm, wu_hbm) if hop is hop1 else (wg_v, wu_v)
            _when(_in_range(j, 0, NP, lo, hi), lambda: op(hop(a, j, j)))
            _when(_in_range(j, NP, NS, lo, hi), lambda: op(hop(b, j - NP, j)))

        def smem_tick(j, lo, hi):
            s_op(j, lo, hi, hop1, wait)
            s_op(j, lo, hi, hop2, start_hi)
            s_op(j - 1, lo - 1, hi - 1, hop2, wait)
            s_op(j + S - 1, lo + S - 1, hi + S - 1, hop1, start_hi)

        def gu_tail_copy():
            rs = pl.ds(D - 8 * gu_tail, 8 * gu_tail)
            return pltpu.make_async_copy(wu_hbm.at[rs], wu_v.at[rs], sems.at[NSEM - 1])

        wd_cps = []
        r = wd_pre
        for i, rows in enumerate(wd_chunks):
            wd_cps.append(pltpu.make_async_copy(wd_hbm.at[pl.ds(r, rows)], wd_v.at[pl.ds(r, rows)],
                                                sems.at[o_wd + i]))
            r += rows

        def issue_kv(b, j, lo, hi):
            slot = _mod2(b, NB)
            _when(_in_range(b, 0, NBLK, lo, hi), lambda: kv_op(kt_hbm, b, slot, j, start_lo))
            _when(_in_range(b, NBLK, 2 * NBLK, lo, hi), lambda: kv_op(vt_hbm, b - NBLK, slot, j, start_lo))
            if j == n - 1:
                def tail():
                    if gu_tail:
                        start_lo(gu_tail_copy())
                    for cp in wd_cps:
                        start_lo(cp)
                _when(_in_range(b, 2 * NBLK - 1, 2 * NBLK, lo, hi), tail)

        def issue_lo(u):
            if u < NI:
                start_lo(init_copy(u))
            else:
                b, j = (u - NI) // n, (u - NI) % n
                issue_kv(b, j, b, b)

        def step_pre(tau, j, lo, hi, tick, ph):
            kv_op(kt_hbm, 0, _mod2(tau, NB), j, wait)
            for si, s in enumerate(slots):
                if s[:2] == (j, 0):
                    trickle(tau + 1, si, lo + 1, hi + 1, start_hi)
            db, jn = (j + LAT) // n, (j + LAT) % n
            issue_kv(tau + db, jn, lo + db, hi + db)
            if not any(s[:2] == (j, 1) for s in slots):
                for si, s in enumerate(slots):
                    if s[0] == j:
                        trickle(tau, si, lo, hi, wait)
            tlo, thi = ticks_before(lo), ticks_before(hi)
            for p, js in enumerate(sched):
                if j in js:
                    k = js.index(j)
                    _when(True if sper == 1 else ph == p,
                          lambda k=k: smem_tick(tick + k, tlo + k, thi + k))

        def step_post(tau, j, lo, hi):
            if any(s[:2] == (j, 1) for s in slots):
                for si, s in enumerate(slots):
                    if s[0] == j:
                        trickle(tau, si, lo, hi, wait)
                for si, s in enumerate(slots):
                    if s[:2] == (j, 1):
                        trickle(tau + 1, si, lo + 1, hi + 1, start_hi)

        def next_tick(tick, ph):
            inc = len(sched[-1])
            for p in range(sper - 1):
                if len(sched[p]) != len(sched[-1]):
                    inc = jnp.where(ph == p, len(sched[p]), inc)
            return (tick + inc, jnp.where(ph == sper - 1, 0, ph + 1))

        cp_c = pltpu.make_async_copy(c_hbm, c_v, sems.at[o_misc])
        cp_x = pltpu.make_async_copy(x_hbm, x_v, sems.at[o_misc + 1])

        mark('p0_issue')
        issue_lo(0)
        start_hi(cp_c)
        start_hi(cp_x)
        for u in range(1, LAT):
            issue_lo(u)
            if u == 3:
                for j in range(S - 1):
                    s_op(j, j, j, hop1, start_hi)

        mark('p1_init')
        s_ref[...] = jnp.zeros_like(s_ref)
        cp_c.wait()
        cp_x.wait()
        c32 = jnp.broadcast_to(c_v[...].astype(jnp.float32), (8, D))
        sc = (c32 * jax.nn.sigmoid(c32)).astype(jnp.bfloat16)
        x32 = jnp.broadcast_to(x_v[...].astype(jnp.float32), (8, D))
        ln1 = _layernorm(x32)

        row = lax.broadcasted_iota(jnp.int32, (8, BR), 0)
        col = lax.broadcasted_iota(jnp.int32, (8, BR), 1)

        def head_mask(bg):
            gcol = col + bg * BR
            return jnp.logical_and(gcol >= row * DH, gcol < (row + 1) * DH)

        big_slots = [si for si, s in enumerate(slots) if s[2] == 'b']
        for u in range(NI):
            init_copy(u).wait()
            for i, si in enumerate(big_slots):
                if (i * NI) // nbig == u:
                    trickle(0, si, 0, 0, start_hi)
            issue_lo(u + LAT)
            if u == NI // 2:
                smem_tick(0, 0, 0)
        mod_a = jnp.dot(sc, wma_v[...], preferred_element_type=jnp.float32)
        h = (ln1 * (1.0 + mod_a[:, D:2 * D]) + mod_a[:, 0:D]).astype(jnp.bfloat16)

        def q_block(b, bg):
            q = jnp.dot(h, wq_v[_mod2(b, 2)], preferred_element_type=jnp.float32)
            qbd[...] = jnp.where(head_mask(bg), q, 0.0).astype(jnp.bfloat16)

        mark('p3_tau0')
        for j in range(n):
            step_pre(0, j, 0, 0, ticks_before(0), 0)
            step_post(0, j, 0, 0)
        q_block(0, 0)

        def k_body(tau, carry):
            tick, ph, g, bg = carry
            slot = _mod2(tau - 1, NB)
            qb = qbd[...]
            for j in range(n):
                step_pre(tau, j, 1, NBLK, tick, ph)
                cs = pl.ds(j * CW, CW)
                s_ref[:, cs] += jnp.dot(qb, kv[slot, :, cs], preferred_element_type=jnp.float32)
                step_post(tau, j, 1, NBLK)
            last = bg == BPG - 1
            bg_next = jnp.where(last, 0, bg + 1)

            @pl.when(tau < NBLK)
            def _():
                q_block(tau, bg_next)

            @pl.when(last)
            def _():
                sg = s_ref[...] * scale
                m = jnp.max(sg, axis=-1, keepdims=True)
                e = jnp.exp(sg - m)
                l = jnp.sum(e, axis=-1, keepdims=True)
                p_ref[g] = e.astype(jnp.bfloat16)
                linv_ref[g] = jnp.broadcast_to(1.0 / l, (8, BR))
                s_ref[...] = jnp.zeros_like(s_ref)
            return next_tick(tick, ph) + (jnp.where(last, g + 1, g), bg_next)

        i32 = lambda v: jnp.int32(v)
        mark('p4_kloop')
        lax.fori_loop(1, NBLK + 1, k_body, (i32(ticks_before(1)), i32(1 % sper), i32(0), i32(0)))

        def v_block(t, g, bg, acc, pre, post):
            slot = _mod2(t, NB)
            o = jnp.zeros((8, BR), jnp.float32)
            for j in range(n):
                pre(j)
                cs = pl.ds(j * CW, CW)
                o = o + lax.dot_general(p_ref[g, :, cs], kv[slot, :, cs], (((1,), (1,)), ((), ())),
                                        preferred_element_type=jnp.float32)
                post(j)
            o = jnp.where(head_mask(bg), o * linv_ref[g], 0.0).astype(jnp.bfloat16)
            return acc + jnp.dot(o, wo_v[_mod2(t, 4)], preferred_element_type=jnp.float32)

        def v_body(tau, carry):
            tick, ph, g, bg, acc = carry
            lo, hi = NBLK + 1, 2 * NBLK - 1
            acc = v_block(tau - 1, g, bg, acc, lambda j: step_pre(tau, j, lo, hi, tick, ph),
                          lambda j: step_post(tau, j, lo, hi))

            @pl.when(jnp.logical_and(tau >= tau_mb, tau < tau_mb + 4))
            def _():
                ch = tau - tau_mb
                modb_ref[ch] = jnp.dot(sc, wmb_v[ch], preferred_element_type=jnp.float32)
            last = bg == BPG - 1
            return next_tick(tick, ph) + (jnp.where(last, g + 1, g), jnp.where(last, 0, bg + 1), acc)

        mark('p6_vloop')
        carry = lax.fori_loop(NBLK + 1, 2 * NBLK, v_body,
                              (i32(ticks_before(NBLK + 1)), i32((NBLK + 1) % sper), i32(0), i32(0),
                               jnp.zeros((8, D), jnp.float32)))

        mark('p7_lastv')
        acc = v_block(2 * NBLK - 1, NG - 1, BPG - 1, carry[4], lambda j: None, lambda j: None)
        mark('p8_ln_gu')
        attn = jnp.broadcast_to(jnp.sum(acc, axis=0, keepdims=True), (8, D))

        x1 = x32 + modb_ref[0] * attn
        h2 = (_layernorm(x1) * (1.0 + modb_ref[2]) + modb_ref[1]).astype(jnp.bfloat16)
        gg = jnp.dot(h2, wg_v[...], preferred_element_type=jnp.float32)
        if gu_tail:
            gu_tail_copy().wait()
        uu = jnp.dot(h2, wu_v[...], preferred_element_type=jnp.float32)
        hh = (gg * uu).astype(jnp.bfloat16)
        mark('p9_wd')
        y = jnp.zeros((8, D), jnp.float32)
        for si in range(nsl):
            trickle(2 * NBLK, si, 2 * NBLK, 2 * NBLK, wait)
        r = 0
        for i, (cp, rows) in enumerate(zip(wd_cps, wd_chunks)):
            cp.wait()
            if i == 0:
                rows += wd_pre
            y = y + jnp.dot(hh[:, r:r + rows], wd_v[r:r + rows, :], preferred_element_type=jnp.float32)
            r += rows
        out = x1 + modb_ref[3] * y
        out_ref[...] = out[0:1, :].astype(out_ref.dtype)
        mark(None)

    scratch = [
        pltpu.VMEM((1, D), jnp.bfloat16),
        pltpu.VMEM((1, D), jnp.bfloat16),
        pltpu.VMEM((D, 2 * D), jnp.bfloat16),
        pltpu.VMEM((4, D, D), jnp.bfloat16),
        pltpu.VMEM((2, D, BR), jnp.bfloat16),
        pltpu.VMEM((4, BR, D), jnp.bfloat16),
        pltpu.VMEM((D, F), jnp.bfloat16),
        pltpu.VMEM((D, F), jnp.bfloat16),
        pltpu.VMEM((F, D), jnp.bfloat16),
        pltpu.VMEM((NB, BR, W), jnp.bfloat16),
        pltpu.VMEM((8, BR), jnp.bfloat16),
        pltpu.VMEM((8, W), jnp.float32),
        pltpu.VMEM((NG, 8, W), jnp.bfloat16),
        pltpu.VMEM((NG, 8, BR), jnp.float32),
        pltpu.VMEM((4, 8, D), jnp.float32),
        pltpu.SMEM((S, 8, F), jnp.bfloat16),
        pltpu.SemaphoreType.DMA((NSEM,)),
    ]
    return kernel, scratch


@jax.jit
def pallas_adaLN_cond__sliding_block_cached__glu_gated_bilinear__decode_kernel(
    A_x: jax.Array,
    A_k_cache: jax.Array,
    A_v_cache: jax.Array,
    A_wq: jax.Array,
    A_wo: jax.Array,
    B_x: jax.Array,
    B_w_gate: jax.Array,
    B_w_up: jax.Array,
    B_w_down: jax.Array,
    c: jax.Array,
    w_mod: jax.Array,
):
    SK = A_k_cache.shape[2]
    W = min(4096, max(256, SK // 4))
    kt = jnp.swapaxes(A_k_cache, 2, 3).reshape(ROWS, SK)
    vt = jnp.swapaxes(A_v_cache, 2, 3).reshape(ROWS, SK)
    kernel, scratch = make_kernel(SK, W, tiles=[[(0, 64, 256, 1024)], [(64, 64, 256, 1024)], [(0, 128, 1280, 256), (0, 128, 1536, 256)], [(0, 128, 1792, 256), (0, 128, 2048, 256)], [(0, 64, 2304, 1024)], [(64, 64, 2304, 1024)], [(0, 128, 3328, 256), (0, 128, 3584, 256)], [(0, 128, 3840, 256), (0, 128, 0, 256)]], plan=[('b', ''), ('b', 's'), ('b', ''), ('b', 's'), ('b', ''), ('b', 's'), ('b', ''), ('b', 's')], LAT=16, gu_tail=12)
    out = pl.pallas_call(
        kernel,
        in_specs=[pl.BlockSpec(memory_space=pl.ANY)] * 10,
        out_specs=pl.BlockSpec(memory_space=pltpu.VMEM),
        out_shape=jax.ShapeDtypeStruct((1, D), jnp.bfloat16),
        scratch_shapes=scratch,
        compiler_params=pltpu.CompilerParams(vmem_limit_bytes=64 * 1024 * 1024,
                                             disable_semaphore_checks=True,
                                             disable_bounds_checks=True),
    )(A_x.reshape(1, D), c, w_mod, A_wq, kt, vt, A_wo, B_w_gate, B_w_up, B_w_down)
    return out.reshape(1, 1, D)
```

```python
import jax
import jax.numpy as jnp
from jax import lax
import jax.experimental.pallas as pl
import jax.experimental.pallas.tpu as pltpu

D = 640
HQ = 32
DH = 192
F = 1536
WIN = 4096
EPS = 1e-5
ROWS = HQ * DH
GH = 8
NG = HQ // GH
BR = 128
NBLK = ROWS // BR
BPG = GH * DH // BR
NT = 2 * NBLK
RES = NBLK - BPG
NP = D // 8

HI, LO = 0, 1

TILES = (
    ((0, 64, 256, 1024),),
    ((64, 64, 256, 1024),),
    ((0, 128, 1280, 256), (0, 128, 1536, 256)),
    ((0, 128, 1792, 256), (0, 128, 2048, 256)),
    ((0, 64, 2304, 1024),),
    ((64, 64, 2304, 1024),),
    ((0, 128, 3328, 256), (0, 128, 3584, 256)),
    ((0, 128, 3840, 256), (0, 128, 0, 256)),
)
NSTEP = len(TILES)
CW = WIN // NSTEP
AHEAD = 2
NB = 8
PR = BR // NSTEP

T_MA, T_WQ, T_G1, T_MB, T_WO, T_END = 0, 5, 35, 36, 47, NT - 1
POST = (1, 5)
NSL = NSTEP + len(POST)
MB0 = (T_WO - T_MB) * NSTEP
T_G2 = T_WO + (2 * NP - MB0) // len(POST)

SCHED = ((1, 7), (5,), (3,))
NSTAGE = 4


def _ticks_before(t):
    return sum(len(SCHED[i % len(SCHED)]) for i in range(t))


NS = _ticks_before(NT) - 1
GU_TAIL = 13
T_G3 = T_G2 + (2 * NP - NS - NSTEP - GU_TAIL) // len(POST)
WD_CHUNKS = (512, 512, 256, 128, 128)

_SEM_OF = {}
for _j, _st in enumerate(TILES):
    for _k in range(len(_st)):
        _SEM_OF[(_j, _k)] = len(_SEM_OF)
NKS = len(_SEM_OF)
O_KV = 0
O_HI = O_KV + NB * NKS
O_S1 = O_HI + 2 * NSL
O_S2 = O_S1 + NSTAGE
O_MISC = O_S2 + NSTAGE
O_WD = O_MISC + 3
NSEM = O_WD + len(WD_CHUNKS)

assert sorted((r, c) for st in TILES for (r0, rn, c0, cn) in st
              for r in range(r0, r0 + rn, 8) for c in range(c0, c0 + cn, 128)) == [
    (r, c) for r in range(0, BR, 8) for c in range(0, WIN, 128)]
assert (T_WQ - T_MA) * BR == D and (T_G1 - T_WQ) * NSTEP == 3 * NP and T_END - T_WO == NBLK
assert MB0 + (T_G2 - T_WO) * len(POST) == 2 * NP and T_G2 <= RES + NBLK and T_G3 <= T_END
assert NS + NSTEP + (T_G3 - T_G2) * len(POST) + GU_TAIL == 2 * NP and NP <= NS
assert sum(WD_CHUNKS) == F and NB >= AHEAD + 2


def _layernorm(x):
    m = jnp.mean(x, axis=-1, keepdims=True)
    xc = x - m
    v = jnp.mean(xc * xc, axis=-1, keepdims=True)
    return xc * lax.rsqrt(v + EPS)


def _dot(a, b):
    return jnp.dot(a, b, preferred_element_type=jnp.float32)


def _static(i):
    return isinstance(i, int)


def _rows(start, size):
    return pl.ds(start if _static(start) else pl.multiple_of(start, 8), size)


def _mod2(i, m):
    return i % m if _static(i) else jnp.bitwise_and(i, m - 1)


def _divmod(i, m):
    q = lax.shift_right_logical(i * ((1 << 16) // m + 1), 16)
    return q, i - q * m


def _when_in(t, a, b, lo, hi, fn):
    if b <= a or b <= lo or a > hi:
        return
    if a <= lo and hi < b:
        fn()
    elif a <= lo:
        pl.when(t < b)(fn)
    elif hi < b:
        pl.when(t >= a)(fn)
    else:
        pl.when(jnp.logical_and(t >= a, t < b))(fn)


def _start_hi(cp):
    cp.start(priority=HI)


def _start_lo(cp):
    cp.start(priority=LO)


def _wait(cp):
    cp.wait()


def _kernel(x_hbm, c_hbm, wmod_hbm, wq_hbm, kt_hbm, vt_hbm, wo_hbm, wg_hbm, wu_hbm, wd_hbm,
            out_ref,
            x_v, c_v, wma_v, wmb_v, wq_v, wo_v, wg_v, wu_v, wd_v, kv, h_ref, q_ref, s_ref, p_ref,
            linv_ref, o_ref, stage, sems):
    col0 = kt_hbm.shape[1] - WIN
    copy = pltpu.make_async_copy

    def block_op(t, j, lo, hi, op):
        ring = _mod2(t, NB)

        def tiles(src, b, slot):
            for k, (rt, rn, ct, cn) in enumerate(TILES[j]):
                op(copy(src.at[_rows(b * BR + rt, rn), pl.ds(col0 + ct, cn)],
                        kv.at[slot, pl.ds(rt, rn), pl.ds(ct, cn)],
                        sems.at[O_KV + ring * NKS + _SEM_OF[(j, k)]]))

        _when_in(t, 0, RES, lo, hi, lambda: tiles(vt_hbm, t, t))
        _when_in(t, RES, RES + NBLK, lo, hi, lambda: tiles(kt_hbm, t - RES, RES + ring))
        _when_in(t, RES + NBLK, NT, lo, hi, lambda: tiles(vt_hbm, t - NBLK, RES + ring))

    def piece_op(t, si, lo, hi, op):
        sem = sems.at[O_HI + _mod2(t, 2) * NSL + si]

        def ma_piece():
            rows = _rows((t - T_MA) * BR + si * PR, PR)
            op(copy(wmod_hbm.at[rows, pl.ds(0, 2 * D)], wma_v.at[rows], sem))

        def wq_piece():
            r, c = _divmod((t - T_WQ) * NSTEP + si, 3)
            rows, cols = _rows(r * 8, 8), pl.ds(pl.multiple_of(c * (ROWS // 3), 128), ROWS // 3)
            op(copy(wq_hbm.at[rows, cols], wq_v.at[rows, cols], sem))

        def wu_piece(k):
            rows = _rows((NS - NP + k) * 8, 8)
            op(copy(wu_hbm.at[rows], wu_v.at[rows], sem))

        def mb_piece(r, half):
            rows = _rows(r * 8, 8)
            op(copy(wmod_hbm.at[rows, pl.ds((1 + half) * 2 * D, 2 * D)],
                    wmb_v.at[rows, pl.ds(half * 2 * D, 2 * D)], sem))

        def wo_piece():
            op(copy(wo_hbm.at[_rows((t - T_WO) * BR + si * PR, PR)],
                    wo_v.at[_mod2(t, 4), pl.ds(si * PR, PR)], sem))

        if si < NSTEP:
            _when_in(t, T_MA, T_WQ, lo, hi, ma_piece)
            _when_in(t, T_WQ, T_G1, lo, hi, wq_piece)
            _when_in(t, T_G1, T_MB, lo, hi, lambda: wu_piece(si))
            _when_in(t, T_MB, T_WO, lo, hi,
                     lambda: mb_piece((t - T_MB) * (NSTEP // 2) + si // 2, si % 2))
            _when_in(t, T_WO, T_END, lo, hi, wo_piece)
        else:
            e = si - NSTEP
            _when_in(t, T_WO, T_G2, lo, hi, lambda: mb_piece(MB0 // 2 + t - T_WO, e))
            _when_in(t, T_G2, T_G3, lo, hi, lambda: wu_piece(NSTEP + (t - T_G2) * len(POST) + e))

    def stage_op(i, lo, hi, inbound, op):
        slot = _mod2(i, NSTAGE)

        def hop(hbm, vmem, r):
            if inbound:
                op(copy(hbm.at[_rows(r * 8, 8)], stage.at[slot], sems.at[O_S1 + slot]))
            else:
                op(copy(stage.at[slot], vmem.at[_rows(r * 8, 8)], sems.at[O_S2 + slot]))

        _when_in(i, 0, NP, lo, hi, lambda: hop(wg_hbm, wg_v, i))
        _when_in(i, NP, NS, lo, hi, lambda: hop(wu_hbm, wu_v, i - NP))

    def stage_tick(i, lo, hi):
        stage_op(i, lo, hi, True, _wait)
        stage_op(i, lo, hi, False, _start_hi)
        stage_op(i - 1, lo - 1, hi - 1, False, _wait)
        d = NSTAGE - 1
        stage_op(i + d, lo + d, hi + d, True, _start_hi)

    def tail_copies():
        rows = pl.ds(D - 8 * GU_TAIL, 8 * GU_TAIL)
        cps = [copy(wu_hbm.at[rows], wu_v.at[rows], sems.at[O_MISC + 2])]
        r = 0
        for i, n in enumerate(WD_CHUNKS):
            cps.append(copy(wd_hbm.at[pl.ds(r, n)], wd_v.at[pl.ds(r, n)], sems.at[O_WD + i]))
            r += n
        return cps

    def start_tail():
        for cp in tail_copies():
            _start_lo(cp)

    def step_pre(t, j, lo, hi, tick, ph):
        block_op(t, j, lo, hi, _wait)
        piece_op(t, j, lo, hi, _start_hi)
        block_op(t + AHEAD, j, lo + AHEAD, hi + AHEAD, _start_lo)
        if j == NSTEP - 1:
            _when_in(t + AHEAD, NT - 1, NT, lo + AHEAD, hi + AHEAD, start_tail)
        if not (j in POST and hi >= T_WO):
            piece_op(t - 1, j, lo - 1, hi - 1, _wait)
        for p, js in enumerate(SCHED):
            if j in js:
                k = js.index(j)
                pl.when(ph == p)(lambda k=k: stage_tick(tick + k, _ticks_before(lo) + k,
                                                        _ticks_before(hi) + k))

    def step_post(t, j, lo, hi):
        if j in POST and hi >= T_WO:
            e = NSTEP + POST.index(j)
            piece_op(t - 1, j, lo - 1, hi - 1, _wait)
            piece_op(t - 1, e, lo - 1, hi - 1, _wait)
            piece_op(t, e, lo, hi, _start_hi)

    def next_tick(tick, ph):
        return tick + jnp.where(ph == 0, 2, 1), jnp.where(ph == len(SCHED) - 1, 0, ph + 1)

    cp_c = copy(c_hbm, c_v, sems.at[O_MISC])
    cp_x = copy(x_hbm, x_v, sems.at[O_MISC + 1])
    for u in range(AHEAD * NSTEP):
        t = u // NSTEP
        block_op(t, u % NSTEP, t, t, _start_lo)
        if u == 0:
            _start_hi(cp_c)
            _start_hi(cp_x)
        if u == 3:
            for i in range(NSTAGE - 1):
                stage_op(i, i, i, True, _start_hi)

    s_ref[...] = jnp.zeros_like(s_ref)
    q_ref[...] = jnp.zeros_like(q_ref)
    cp_c.wait()
    cp_x.wait()
    c32 = jnp.broadcast_to(c_v[...].astype(jnp.float32), (GH, D))
    sc = (c32 * jax.nn.sigmoid(c32)).astype(jnp.bfloat16)
    x32 = jnp.broadcast_to(x_v[...].astype(jnp.float32), (GH, D))
    row = lax.broadcasted_iota(jnp.int32, (GH, BR), 0)
    col = lax.broadcasted_iota(jnp.int32, (GH, BR), 1)

    def head_body(t, carry):
        tick, ph = carry
        r, rem = _divmod(t, 6)
        is_q = jnp.logical_and(rem == 0, t >= 12)
        qb = NBLK // NSTEP
        for j in range(NSTEP):
            step_pre(t, j, 0, RES, tick, ph)

            @pl.when(is_q)
            def _():
                res = _dot(h_ref[r - 2],
                           wq_v[_rows((r - 2) * BR, BR), j * qb * BR:(j + 1) * qb * BR])
                for i in range(qb):
                    q_ref[j * qb + i] += res[:, i * BR:(i + 1) * BR]

        @pl.when(t == T_WQ)
        def _():
            mod_a = _dot(sc, wma_v[...])
            h = (_layernorm(x32) * (1.0 + mod_a[:, D:2 * D]) + mod_a[:, 0:D]).astype(jnp.bfloat16)
            for i in range(D // BR):
                h_ref[i] = h[:, i * BR:(i + 1) * BR]
        return next_tick(tick, ph)

    lax.fori_loop(0, RES + 1, head_body, (jnp.int32(0), jnp.int32(0)))

    def attn_block(t, g, bg, acc, do_k, do_v, pre, post):
        ring_slot = RES + _mod2(t - 1, NB)
        gcol = col + bg * BR
        mask = jnp.logical_and(gcol >= row * DH, gcol < (row + 1) * DH)
        both = do_k and do_v
        if do_k:
            q = jnp.where(mask, q_ref[t - RES - 1], 0.0).astype(jnp.bfloat16)
        v_slot = t - NBLK - 1 if both else ring_slot
        for j in range(NSTEP):
            pre(j)
            cs = pl.ds((j // 2) * 2 * CW, 2 * CW) if both else pl.ds(j * CW, CW)
            if do_k and not (both and j % 2 == 0):
                s_ref[:, cs] += _dot(q, kv[ring_slot, :, cs])
            if do_v and not (both and j % 2 == 1):
                part = lax.dot_general(p_ref[g - 1, :, cs], kv[v_slot, :, cs],
                                       (((1,), (1,)), ((), ())),
                                       preferred_element_type=jnp.float32)
                if j == 0:
                    o_ref[...] = part
                else:
                    o_ref[...] += part
            post(j)
        if do_v:
            o = jnp.where(mask, o_ref[...] * linv_ref[g - 1], 0.0).astype(jnp.bfloat16)
            acc = acc + _dot(o, wo_v[_mod2(t - 2, 4)])
        return acc

    def attn_loop(lo, hi, do_k, do_v, acc):
        def body(t, carry):
            tick, ph, g, bg, acc = carry
            acc = attn_block(t, g, bg, acc, do_k, do_v,
                             lambda j: step_pre(t, j, lo, hi, tick, ph),
                             lambda j: step_post(t, j, lo, hi))
            last = bg == BPG - 1
            if do_k:
                @pl.when(last)
                def _():
                    s = s_ref[...] * (DH ** -0.5)
                    e = jnp.exp(s - jnp.max(s, axis=-1, keepdims=True))
                    p_ref[g] = e.astype(jnp.bfloat16)
                    linv_ref[g] = jnp.broadcast_to(1.0 / jnp.sum(e, axis=-1, keepdims=True), (GH, BR))
                    s_ref[...] = jnp.zeros_like(s_ref)
            return next_tick(tick, ph) + (jnp.where(last, g + 1, g), jnp.where(last, 0, bg + 1), acc)

        g0, bg0 = divmod(lo - RES - 1, BPG)
        init = tuple(jnp.int32(v) for v in (_ticks_before(lo), lo % len(SCHED), g0, bg0)) + (acc,)
        return lax.fori_loop(lo, hi + 1, body, init)[4]

    acc = jnp.zeros((GH, D), jnp.float32)
    attn_loop(RES + 1, NBLK, True, False, acc)
    acc = attn_loop(NBLK + 1, RES + NBLK, True, True, acc)
    mod_b = _dot(sc, wmb_v[...])
    acc = attn_loop(RES + NBLK + 1, NT - 1, False, True, acc)
    acc = attn_block(NT, NG, BPG - 1, acc, False, True, lambda j: None, lambda j: None)
    attn = jnp.broadcast_to(jnp.sum(acc, axis=0, keepdims=True), (GH, D))

    tail = tail_copies()
    x1 = x32 + mod_b[:, 0:D] * attn
    h2 = (_layernorm(x1) * (1.0 + mod_b[:, 2 * D:3 * D]) + mod_b[:, D:2 * D]).astype(jnp.bfloat16)
    gate = _dot(h2, wg_v[...])
    tail[0].wait()
    hh = (gate * _dot(h2, wu_v[...])).astype(jnp.bfloat16)
    y = jnp.zeros((GH, D), jnp.float32)
    r = 0
    for cp, n in zip(tail[1:], WD_CHUNKS):
        cp.wait()
        y = y + _dot(hh[:, r:r + n], wd_v[r:r + n, :])
        r += n
    out = x1 + mod_b[:, 3 * D:4 * D] * y
    out_ref[...] = out[0:1, :].astype(out_ref.dtype)


@jax.jit
def pallas_adaLN_cond__sliding_block_cached__glu_gated_bilinear__decode_kernel(
    A_x: jax.Array,
    A_k_cache: jax.Array,
    A_v_cache: jax.Array,
    A_wq: jax.Array,
    A_wo: jax.Array,
    B_x: jax.Array,
    B_w_gate: jax.Array,
    B_w_up: jax.Array,
    B_w_down: jax.Array,
    c: jax.Array,
    w_mod: jax.Array,
):
    sk = A_k_cache.shape[2]
    assert A_k_cache.shape == (1, HQ, sk, DH) and min(4096, max(256, sk // 4)) == WIN
    kt = jnp.swapaxes(A_k_cache, 2, 3).reshape(ROWS, sk)
    vt = jnp.swapaxes(A_v_cache, 2, 3).reshape(ROWS, sk)
    bf16, f32 = jnp.bfloat16, jnp.float32
    out = pl.pallas_call(
        _kernel,
        in_specs=[pl.BlockSpec(memory_space=pl.ANY)] * 10,
        out_specs=pl.BlockSpec(memory_space=pltpu.VMEM),
        out_shape=jax.ShapeDtypeStruct((1, D), A_x.dtype),
        scratch_shapes=[
            pltpu.VMEM((1, D), bf16),
            pltpu.VMEM((1, D), bf16),
            pltpu.VMEM((D, 2 * D), bf16),
            pltpu.VMEM((D, 4 * D), bf16),
            pltpu.VMEM((D, ROWS), bf16),
            pltpu.VMEM((4, BR, D), bf16),
            pltpu.VMEM((D, F), bf16),
            pltpu.VMEM((D, F), bf16),
            pltpu.VMEM((F, D), bf16),
            pltpu.VMEM((RES + NB, BR, WIN), bf16),
            pltpu.VMEM((D // BR, GH, BR), bf16),
            pltpu.VMEM((NBLK, GH, BR), f32),
            pltpu.VMEM((GH, WIN), f32),
            pltpu.VMEM((NG, GH, WIN), bf16),
            pltpu.VMEM((NG, GH, BR), f32),
            pltpu.VMEM((GH, BR), f32),
            pltpu.SMEM((NSTAGE, 8, F), bf16),
            pltpu.SemaphoreType.DMA((NSEM,)),
        ],
        compiler_params=pltpu.CompilerParams(
            vmem_limit_bytes=96 * 1024 * 1024,
            disable_bounds_checks=True,
            disable_semaphore_checks=True,
        ),
    )(A_x.reshape(1, D), c, w_mod, A_wq, kt, vt, A_wo, B_w_gate, B_w_up, B_w_down)
    return out.reshape(1, 1, D)
```

```python
import jax
import jax.numpy as jnp
from jax import lax
import jax.experimental.pallas as pl
import jax.experimental.pallas.tpu as pltpu

D = 640
HQ = 32
DH = 192
F = 1536
WIN = 4096
EPS = 1e-5
ROWS = HQ * DH
GH = 8
NG = HQ // GH
BR = 128
NBLK = ROWS // BR
BPG = GH * DH // BR
NT = 2 * NBLK
RES = NBLK - BPG
NP = D // 8
HI, LO = 0, 1

TILES = (
    tuple((r, 32, 256, 1024) for r in range(0, BR, 32))
    + tuple((0, BR, c, 256) for c in range(1280, 2304, 256))
    + tuple((r, 32, 2304, 1024) for r in range(0, BR, 32))
    + tuple((0, BR, c, 256) for c in (3328, 3584, 3840, 0))
)
NTILE = len(TILES)
NSTEP = NTILE // 2
CW = WIN // NSTEP
AHEAD = 24
NB = 4

T_MA, T_WQ, T_WG, T_U1, T_WO, T_U2, T_WD = 0, 5, 35, 45, 47, 87, NT - 1
U1 = (T_WO - T_U1) * NSTEP
U_TAIL = NP - U1 - (T_WD - T_U2) * NSTEP // 2
WD_PRE = 16 * NTILE
WD_CHUNKS = (256, 512, 256, 128, 128)

O_KV = 0
O_HI = O_KV + NB * NTILE
O_MISC = O_HI + 2 * NTILE
O_WD = O_MISC + 3
NSEM = O_WD + len(WD_CHUNKS)

assert sorted((r, c) for (r0, rn, c0, cn) in TILES
              for r in range(r0, r0 + rn, 8) for c in range(c0, c0 + cn, 128)) == [
    (r, c) for r in range(0, BR, 8) for c in range(0, WIN, 128)]
assert (T_WQ - T_MA) * NTILE == NP and (T_WG - T_WQ) * NTILE == 6 * NP
assert (T_U1 - T_WG) * NSTEP == NP and (T_U2 - T_WO) * 2 == NP and T_WD - T_WO == NBLK
assert WD_PRE + sum(WD_CHUNKS) == F and U_TAIL > 0
assert AHEAD % 2 == 0 and AHEAD + 2 * NTILE <= NB * NTILE
assert all((i * 10923) >> 16 == i // 6 for i in range(6 * NP))


def _layernorm(x):
    m = jnp.mean(x, axis=-1, keepdims=True)
    xc = x - m
    v = jnp.mean(xc * xc, axis=-1, keepdims=True)
    return xc * lax.rsqrt(v + EPS)


def _dot(a, b):
    return jnp.dot(a, b, preferred_element_type=jnp.float32)


def _rows(start, size):
    return pl.ds(start if isinstance(start, int) else pl.multiple_of(start, 8), size)


def _mod2(i, m):
    return i % m if isinstance(i, int) else jnp.bitwise_and(i, m - 1)


def _divmod6(i):
    q = lax.shift_right_logical(i * 10923, 16)
    return q, i - q * 6


def _when_in(t, a, b, lo, hi, fn):
    if b <= lo or a > hi:
        return
    if a <= lo and hi < b:
        fn()
    elif a <= lo:
        pl.when(t < b)(fn)
    elif hi < b:
        pl.when(t >= a)(fn)
    else:
        pl.when(jnp.logical_and(t >= a, t < b))(fn)


def _start_hi(cp):
    cp.start(priority=HI)


def _start_lo(cp):
    cp.start(priority=LO)


def _wait(cp):
    cp.wait()


def _kernel(x_hbm, c_hbm, wmod_hbm, wq_hbm, kt_hbm, vt_hbm, wo_hbm, wg_hbm, wu_hbm, wd_hbm,
            out_ref,
            x_v, c_v, wma_v, wmb_v, wq_v, wo_v, wg_v, wu_v, wd_v, vres, ring, h_ref, q_ref, s_ref,
            p_ref, linv_ref, o_ref, modb_ref, sems):
    col0 = kt_hbm.shape[1] - WIN
    copy = pltpu.make_async_copy

    def tile_op(t, k, lo, hi, op):
        slot = _mod2(t, NB)
        rt, rn, ct, cn = TILES[k]

        def tile(src, b, dst, i):
            op(copy(src.at[_rows(b * BR + rt, rn), pl.ds(col0 + ct, cn)],
                    dst.at[i, pl.ds(rt, rn), pl.ds(ct, cn)], sems.at[O_KV + slot * NTILE + k]))

        _when_in(t, 0, RES, lo, hi, lambda: tile(vt_hbm, t, vres, t))
        _when_in(t, RES, RES + NBLK, lo, hi, lambda: tile(kt_hbm, t - RES, ring, slot))
        _when_in(t, RES + NBLK, NT, lo, hi, lambda: tile(vt_hbm, t - NBLK, ring, slot))

    def piece_op(t, k, lo, hi, op):
        sem = sems.at[O_HI + _mod2(t, 2) * NTILE + k]
        j, odd = divmod(k, 2)
        hf = F // 2

        def same(src, dst, r, c0, cn):
            rows, cols = _rows(r * 8, 8), pl.ds(c0, cn)
            op(copy(src.at[rows, cols], dst.at[rows, cols], sem))

        def wq_piece():
            r, c = _divmod6((t - T_WQ) * NTILE + k)
            same(wq_hbm, wq_v, r, pl.multiple_of(c * (ROWS // 6), 128), ROWS // 6)

        def wo_piece():
            op(copy(wo_hbm.at[_rows((t - T_WO) * BR + j * 16, 16)],
                    wo_v.at[_mod2(t, 4), pl.ds(j * 16, 16)], sem))

        def mb_piece():
            rows = _rows((t - T_WO) * 16 + (j // 4) * 8, 8)
            op(copy(wmod_hbm.at[rows, pl.ds((2 + j % 4) * D, D)],
                    wmb_v.at[rows, pl.ds((j % 4) * D, D)], sem))

        def wd_piece():
            op(copy(wd_hbm.at[pl.ds(k * 16, 16)], wd_v.at[pl.ds(k * 16, 16)], sem))

        _when_in(t, T_MA, T_WQ, lo, hi,
                 lambda: same(wmod_hbm, wma_v, (t - T_MA) * NTILE + k, 0, 2 * D))
        _when_in(t, T_WQ, T_WG, lo, hi, wq_piece)
        _when_in(t, T_WG, T_U1, lo, hi,
                 lambda: same(wg_hbm, wg_v, (t - T_WG) * NSTEP + j, odd * hf, hf))
        _when_in(t, T_U1, T_WO, lo, hi,
                 lambda: same(wu_hbm, wu_v, (t - T_U1) * NSTEP + j, odd * hf, hf))
        if odd:
            _when_in(t, T_WO, T_U2, lo, hi, mb_piece)
            _when_in(t, T_U2, T_WD, lo, hi,
                     lambda: same(wu_hbm, wu_v, U1 + (t - T_U2) * (NSTEP // 2) + j // 2,
                                  (j % 2) * hf, hf))
        else:
            _when_in(t, T_WO, T_WD, lo, hi, wo_piece)
        _when_in(t, T_WD, NT, lo, hi, wd_piece)

    def tail_copies():
        rows = pl.ds(D - 8 * U_TAIL, 8 * U_TAIL)
        cps = [copy(wu_hbm.at[rows], wu_v.at[rows], sems.at[O_MISC + 2])]
        r = WD_PRE
        for i, n in enumerate(WD_CHUNKS):
            cps.append(copy(wd_hbm.at[pl.ds(r, n)], wd_v.at[pl.ds(r, n)], sems.at[O_WD + i]))
            r += n
        return cps

    def start_tail():
        for cp in tail_copies():
            _start_lo(cp)

    def step_open(t, j, lo, hi):
        tile_op(t, 2 * j, lo, hi, _wait)
        piece_op(t, 2 * j, lo, hi, _start_hi)

    def step_close(t, j, lo, hi):
        db, k = divmod(2 * j + AHEAD, NTILE)
        tile_op(t + db, k, lo + db, hi + db, _start_lo)
        tile_op(t + db, k + 1, lo + db, hi + db, _start_lo)
        if k + 2 == NTILE:
            _when_in(t + db, NT - 1, NT, lo + db, hi + db, start_tail)
        tile_op(t, 2 * j + 1, lo, hi, _wait)
        piece_op(t - 1, 2 * j, lo - 1, hi - 1, _wait)
        piece_op(t - 1, 2 * j + 1, lo - 1, hi - 1, _wait)
        piece_op(t, 2 * j + 1, lo, hi, _start_hi)

    cp_c = copy(c_hbm, c_v, sems.at[O_MISC])
    cp_x = copy(x_hbm, x_v, sems.at[O_MISC + 1])
    for u in range(AHEAD):
        t, k = divmod(u, NTILE)
        tile_op(t, k, t, t, _start_lo)
        if u == 0:
            _start_hi(cp_c)
            _start_hi(cp_x)

    s_ref[...] = jnp.zeros_like(s_ref)
    q_ref[...] = jnp.zeros_like(q_ref)
    cp_c.wait()
    cp_x.wait()
    c32 = jnp.broadcast_to(c_v[...].astype(jnp.float32), (GH, D))
    sc = (c32 * jax.nn.sigmoid(c32)).astype(jnp.bfloat16)
    x32 = jnp.broadcast_to(x_v[...].astype(jnp.float32), (GH, D))
    row = lax.broadcasted_iota(jnp.int32, (GH, BR), 0)
    col = lax.broadcasted_iota(jnp.int32, (GH, BR), 1)

    def head_body(t, carry):
        r, rem = _divmod6(t)
        is_q = jnp.logical_and(rem == 0, t >= 12)
        qb = NBLK // NSTEP
        for j in range(NSTEP):
            step_open(t, j, 0, RES)

            @pl.when(is_q)
            def _():
                res = _dot(h_ref[r - 2],
                           wq_v[_rows((r - 2) * BR, BR), j * qb * BR:(j + 1) * qb * BR])
                for i in range(qb):
                    q_ref[j * qb + i] += res[:, i * BR:(i + 1) * BR]

            step_close(t, j, 0, RES)

        @pl.when(t == T_WQ)
        def _():
            mod_a = _dot(sc, wma_v[...])
            h = (_layernorm(x32) * (1.0 + mod_a[:, D:2 * D]) + mod_a[:, 0:D]).astype(jnp.bfloat16)
            for i in range(D // BR):
                h_ref[i] = h[:, i * BR:(i + 1) * BR]
        return carry

    lax.fori_loop(0, RES + 1, head_body, 0)

    def attn_block(t, g, bg, acc, do_k, do_v, opener, closer):
        slot = _mod2(t - 1, NB)
        gcol = col + bg * BR
        mask = jnp.logical_and(gcol >= row * DH, gcol < (row + 1) * DH)
        both = do_k and do_v
        if do_k:
            q = jnp.where(mask, q_ref[t - RES - 1], 0.0).astype(jnp.bfloat16)
        v_buf, v_slot = (vres, t - NBLK - 1) if both else (ring, slot)
        for j in range(NSTEP):
            opener(j)
            cs = pl.ds((j // 2) * 2 * CW, 2 * CW) if both else pl.ds(j * CW, CW)
            if do_k and not (both and j % 2 == 0):
                s_ref[:, cs] += _dot(q, ring[slot, :, cs])
            else:
                part = lax.dot_general(p_ref[g - 1, :, cs], v_buf[v_slot, :, cs],
                                       (((1,), (1,)), ((), ())),
                                       preferred_element_type=jnp.float32)
                if j == 0:
                    o_ref[...] = part
                else:
                    o_ref[...] += part
            closer(j)
        if do_v:
            o = jnp.where(mask, o_ref[...] * linv_ref[g - 1], 0.0).astype(jnp.bfloat16)
            acc = acc + _dot(o, wo_v[_mod2(t - 2, 4)])
        return acc

    def attn_loop(lo, hi, do_k, do_v, acc):
        def body(t, carry):
            g, bg, acc = carry
            acc = attn_block(t, g, bg, acc, do_k, do_v,
                             lambda j: step_open(t, j, lo, hi), lambda j: step_close(t, j, lo, hi))
            last = bg == BPG - 1
            if do_k:
                @pl.when(last)
                def _():
                    s = s_ref[...] * (DH ** -0.5)
                    e = jnp.exp(s - jnp.max(s, axis=-1, keepdims=True))
                    p_ref[g] = e.astype(jnp.bfloat16)
                    linv_ref[g] = jnp.broadcast_to(1.0 / jnp.sum(e, axis=-1, keepdims=True), (GH, BR))
                    s_ref[...] = jnp.zeros_like(s_ref)
            else:
                for ch in range(4):
                    @pl.when(t == T_U2 + 1 + ch)
                    def _():
                        modb_ref[ch] = _dot(sc, wmb_v[:, ch * D:(ch + 1) * D])
            return jnp.where(last, g + 1, g), jnp.where(last, 0, bg + 1), acc

        g0, bg0 = divmod(lo - RES - 1, BPG)
        return lax.fori_loop(lo, hi + 1, body, (jnp.int32(g0), jnp.int32(bg0), acc))[2]

    acc = jnp.zeros((GH, D), jnp.float32)
    attn_loop(RES + 1, NBLK, True, False, acc)
    acc = attn_loop(NBLK + 1, RES + NBLK, True, True, acc)
    acc = attn_loop(RES + NBLK + 1, NT - 1, False, True, acc)
    acc = attn_block(NT, NG, BPG - 1, acc, False, True, lambda j: None, lambda j: None)
    attn = jnp.broadcast_to(jnp.sum(acc, axis=0, keepdims=True), (GH, D))

    tail = tail_copies()
    x1 = x32 + modb_ref[0] * attn
    h2 = (_layernorm(x1) * (1.0 + modb_ref[2]) + modb_ref[1]).astype(jnp.bfloat16)
    gate = _dot(h2, wg_v[...])
    tail[0].wait()
    hh = (gate * _dot(h2, wu_v[...])).astype(jnp.bfloat16)
    for k in range(NTILE):
        piece_op(T_WD, k, T_WD, T_WD, _wait)
    y = jnp.zeros((GH, D), jnp.float32)
    r0, r1 = 0, WD_PRE
    for cp, n in zip(tail[1:], WD_CHUNKS):
        cp.wait()
        r1 += n
        y = y + _dot(hh[:, r0:r1], wd_v[r0:r1, :])
        r0 = r1
    out = x1 + modb_ref[3] * y
    out_ref[...] = out[0:1, :].astype(out_ref.dtype)


@jax.jit
def pallas_adaLN_cond__sliding_block_cached__glu_gated_bilinear__decode_kernel(
    A_x: jax.Array,
    A_k_cache: jax.Array,
    A_v_cache: jax.Array,
    A_wq: jax.Array,
    A_wo: jax.Array,
    B_x: jax.Array,
    B_w_gate: jax.Array,
    B_w_up: jax.Array,
    B_w_down: jax.Array,
    c: jax.Array,
    w_mod: jax.Array,
):
    sk = A_k_cache.shape[2]
    assert A_k_cache.shape == (1, HQ, sk, DH) and min(4096, max(256, sk // 4)) == WIN
    kt = jnp.swapaxes(A_k_cache, 2, 3).reshape(ROWS, sk)
    vt = jnp.swapaxes(A_v_cache, 2, 3).reshape(ROWS, sk)
    bf16, f32 = jnp.bfloat16, jnp.float32
    out = pl.pallas_call(
        _kernel,
        in_specs=[pl.BlockSpec(memory_space=pl.ANY)] * 10,
        out_specs=pl.BlockSpec(memory_space=pltpu.VMEM),
        out_shape=jax.ShapeDtypeStruct((1, D), A_x.dtype),
        scratch_shapes=[
            pltpu.VMEM((1, D), bf16),
            pltpu.VMEM((1, D), bf16),
            pltpu.VMEM((D, 2 * D), bf16),
            pltpu.VMEM((D, 4 * D), bf16),
            pltpu.VMEM((D, ROWS), bf16),
            pltpu.VMEM((4, BR, D), bf16),
            pltpu.VMEM((D, F), bf16),
            pltpu.VMEM((D, F), bf16),
            pltpu.VMEM((F, D), bf16),
            pltpu.VMEM((RES, BR, WIN), bf16),
            pltpu.VMEM((NB, BR, WIN), bf16),
            pltpu.VMEM((D // BR, GH, BR), bf16),
            pltpu.VMEM((NBLK, GH, BR), f32),
            pltpu.VMEM((GH, WIN), f32),
            pltpu.VMEM((NG, GH, WIN), bf16),
            pltpu.VMEM((NG, GH, BR), f32),
            pltpu.VMEM((GH, BR), f32),
            pltpu.VMEM((4, GH, D), f32),
            pltpu.SemaphoreType.DMA((NSEM,)),
        ],
        compiler_params=pltpu.CompilerParams(
            vmem_limit_bytes=96 * 1024 * 1024,
            disable_bounds_checks=True,
            disable_semaphore_checks=True,
        ),
    )(A_x.reshape(1, D), c, w_mod, A_wq, kt, vt, A_wo, B_w_gate, B_w_up, B_w_down)
    return out.reshape(1, 1, D)
```

```python
import jax
import jax.numpy as jnp
from jax import lax
import jax.experimental.pallas as pl
import jax.experimental.pallas.tpu as pltpu

D = 640
HQ = 32
DH = 192
F = 1536
WIN = 4096
EPS = 1e-5
ROWS = HQ * DH
GH = 8
NG = HQ // GH
BR = 128
NBLK = ROWS // BR
BPG = GH * DH // BR
NT = 2 * NBLK
RES = NBLK - BPG
NP = D // 8
HI, LO = 0, 1

TILES = (
    tuple((r, 32, 256, 1024) for r in range(0, BR, 32))
    + tuple((0, BR, c, 256) for c in range(1280, 2304, 256))
    + tuple((r, 32, 2304, 1024) for r in range(0, BR, 32))
    + tuple((0, BR, c, 256) for c in (3328, 3584, 3840, 0))
)
NTILE = len(TILES)
NSTEP = NTILE // 2
CW = WIN // NSTEP
AHEAD = 24
NB = 4

T_MA, T_WQ, T_WG, T_U1, T_WO, T_U2, T_WD = 0, 5, 35, 45, 47, 87, NT - 1
U1 = (T_WO - T_U1) * NSTEP
U_TAIL = NP - U1 - (T_WD - T_U2) * NSTEP // 2
WD_PRE = 16 * NTILE
WD_MXU = (256, 512, 256, 128)
WD_VPU = (96, 32)
WD_CHUNKS = WD_MXU + WD_VPU

O_KV = 0
O_HI = O_KV + NB * NTILE
O_MISC = O_HI + 2 * NTILE
O_WD = O_MISC + 3
NSEM = O_WD + len(WD_CHUNKS)

assert sorted((r, c) for (r0, rn, c0, cn) in TILES
              for r in range(r0, r0 + rn, 8) for c in range(c0, c0 + cn, 128)) == [
    (r, c) for r in range(0, BR, 8) for c in range(0, WIN, 128)]
assert (T_WQ - T_MA) * NTILE == NP and (T_WG - T_WQ) * NTILE == 6 * NP
assert (T_U1 - T_WG) * NSTEP == NP and (T_U2 - T_WO) * 2 == NP and T_WD - T_WO == NBLK
assert WD_PRE + sum(WD_CHUNKS) == F and sum(WD_VPU) == BR and U_TAIL > 0
assert AHEAD % 2 == 0 and AHEAD + 2 * NTILE <= NB * NTILE
assert all((i * 10923) >> 16 == i // 6 for i in range(6 * NP))


def _layernorm(x):
    m = jnp.mean(x, axis=-1, keepdims=True)
    xc = x - m
    v = jnp.mean(xc * xc, axis=-1, keepdims=True)
    return xc * lax.rsqrt(v + EPS)


def _dot(a, b):
    return jnp.dot(a, b, preferred_element_type=jnp.float32)


def _rows(start, size):
    return pl.ds(start if isinstance(start, int) else pl.multiple_of(start, 8), size)


def _mod2(i, m):
    return i % m if isinstance(i, int) else jnp.bitwise_and(i, m - 1)


def _divmod6(i):
    q = lax.shift_right_logical(i * 10923, 16)
    return q, i - q * 6


def _when_in(t, a, b, lo, hi, fn):
    if b <= lo or a > hi:
        return
    if a <= lo and hi < b:
        fn()
    elif a <= lo:
        pl.when(t < b)(fn)
    elif hi < b:
        pl.when(t >= a)(fn)
    else:
        pl.when(jnp.logical_and(t >= a, t < b))(fn)


def _start_hi(cp):
    cp.start(priority=HI)


def _start_lo(cp):
    cp.start(priority=LO)


def _wait(cp):
    cp.wait()


def _kernel(x_hbm, c_hbm, wmod_hbm, wq_hbm, kt_hbm, vt_hbm, wo_hbm, wg_hbm, wu_hbm, wd_hbm,
            out_ref,
            x_v, c_v, wma_v, wmb_v, wq_v, wo_v, wg_v, wu_v, wd_v, vres, ring, h_ref, q_ref, s_ref,
            p_ref, linv_ref, o_ref, modb_ref, sems):
    col0 = kt_hbm.shape[1] - WIN
    copy = pltpu.make_async_copy

    def tile_op(t, k, lo, hi, op):
        slot = _mod2(t, NB)
        rt, rn, ct, cn = TILES[k]

        def tile(src, b, dst, i):
            op(copy(src.at[_rows(b * BR + rt, rn), pl.ds(col0 + ct, cn)],
                    dst.at[i, pl.ds(rt, rn), pl.ds(ct, cn)], sems.at[O_KV + slot * NTILE + k]))

        _when_in(t, 0, RES, lo, hi, lambda: tile(vt_hbm, t, vres, t))
        _when_in(t, RES, RES + NBLK, lo, hi, lambda: tile(kt_hbm, t - RES, ring, slot))
        _when_in(t, RES + NBLK, NT, lo, hi, lambda: tile(vt_hbm, t - NBLK, ring, slot))

    def piece_op(t, k, lo, hi, op):
        sem = sems.at[O_HI + _mod2(t, 2) * NTILE + k]
        j, odd = divmod(k, 2)
        hf = F // 2

        def same(src, dst, r, c0, cn):
            rows, cols = _rows(r * 8, 8), pl.ds(c0, cn)
            op(copy(src.at[rows, cols], dst.at[rows, cols], sem))

        def wq_piece():
            r, c = _divmod6((t - T_WQ) * NTILE + k)
            same(wq_hbm, wq_v, r, pl.multiple_of(c * (ROWS // 6), 128), ROWS // 6)

        def wo_piece():
            op(copy(wo_hbm.at[_rows((t - T_WO) * BR + j * 16, 16)],
                    wo_v.at[_mod2(t, 4), pl.ds(j * 16, 16)], sem))

        def mb_piece():
            rows = _rows((t - T_WO) * 16 + (j // 4) * 8, 8)
            op(copy(wmod_hbm.at[rows, pl.ds((2 + j % 4) * D, D)],
                    wmb_v.at[rows, pl.ds((j % 4) * D, D)], sem))

        def wd_piece():
            op(copy(wd_hbm.at[pl.ds(k * 16, 16)], wd_v.at[pl.ds(k * 16, 16)], sem))

        _when_in(t, T_MA, T_WQ, lo, hi,
                 lambda: same(wmod_hbm, wma_v, (t - T_MA) * NTILE + k, 0, 2 * D))
        _when_in(t, T_WQ, T_WG, lo, hi, wq_piece)
        _when_in(t, T_WG, T_U1, lo, hi,
                 lambda: same(wg_hbm, wg_v, (t - T_WG) * NSTEP + j, odd * hf, hf))
        _when_in(t, T_U1, T_WO, lo, hi,
                 lambda: same(wu_hbm, wu_v, (t - T_U1) * NSTEP + j, odd * hf, hf))
        if odd:
            _when_in(t, T_WO, T_U2, lo, hi, mb_piece)
            _when_in(t, T_U2, T_WD, lo, hi,
                     lambda: same(wu_hbm, wu_v, U1 + (t - T_U2) * (NSTEP // 2) + j // 2,
                                  (j % 2) * hf, hf))
        else:
            _when_in(t, T_WO, T_WD, lo, hi, wo_piece)
        _when_in(t, T_WD, NT, lo, hi, wd_piece)

    def tail_copies():
        rows = pl.ds(D - 8 * U_TAIL, 8 * U_TAIL)
        cps = [copy(wu_hbm.at[rows], wu_v.at[rows], sems.at[O_MISC + 2])]
        r = WD_PRE
        for i, n in enumerate(WD_CHUNKS):
            cps.append(copy(wd_hbm.at[pl.ds(r, n)], wd_v.at[pl.ds(r, n)], sems.at[O_WD + i]))
            r += n
        return cps

    def start_tail():
        for cp in tail_copies():
            _start_lo(cp)

    def step_open(t, j, lo, hi):
        tile_op(t, 2 * j, lo, hi, _wait)
        piece_op(t, 2 * j, lo, hi, _start_hi)

    def step_close(t, j, lo, hi):
        db, k = divmod(2 * j + AHEAD, NTILE)
        tile_op(t + db, k, lo + db, hi + db, _start_lo)
        tile_op(t + db, k + 1, lo + db, hi + db, _start_lo)
        if k + 2 == NTILE:
            _when_in(t + db, NT - 1, NT, lo + db, hi + db, start_tail)
        tile_op(t, 2 * j + 1, lo, hi, _wait)
        piece_op(t - 1, 2 * j, lo - 1, hi - 1, _wait)
        piece_op(t - 1, 2 * j + 1, lo - 1, hi - 1, _wait)
        piece_op(t, 2 * j + 1, lo, hi, _start_hi)

    cp_c = copy(c_hbm, c_v, sems.at[O_MISC])
    cp_x = copy(x_hbm, x_v, sems.at[O_MISC + 1])
    for u in range(AHEAD):
        t, k = divmod(u, NTILE)
        tile_op(t, k, t, t, _start_lo)
        if u == 0:
            _start_hi(cp_c)
            _start_hi(cp_x)

    s_ref[...] = jnp.zeros_like(s_ref)
    q_ref[...] = jnp.zeros_like(q_ref)
    cp_c.wait()
    cp_x.wait()
    c32 = jnp.broadcast_to(c_v[...].astype(jnp.float32), (GH, D))
    sc = (c32 * jax.nn.sigmoid(c32)).astype(jnp.bfloat16)
    x32 = jnp.broadcast_to(x_v[...].astype(jnp.float32), (GH, D))
    row = lax.broadcasted_iota(jnp.int32, (GH, BR), 0)
    col = lax.broadcasted_iota(jnp.int32, (GH, BR), 1)

    def head_body(t, carry):
        r, rem = _divmod6(t)
        is_q = jnp.logical_and(rem == 0, t >= 12)
        qb = NBLK // NSTEP
        for j in range(NSTEP):
            step_open(t, j, 0, RES)

            @pl.when(is_q)
            def _():
                res = _dot(h_ref[r - 2],
                           wq_v[_rows((r - 2) * BR, BR), j * qb * BR:(j + 1) * qb * BR])
                for i in range(qb):
                    q_ref[j * qb + i] += res[:, i * BR:(i + 1) * BR]

            step_close(t, j, 0, RES)

        @pl.when(t == T_WQ)
        def _():
            mod_a = _dot(sc, wma_v[...])
            h = (_layernorm(x32) * (1.0 + mod_a[:, D:2 * D]) + mod_a[:, 0:D]).astype(jnp.bfloat16)
            for i in range(D // BR):
                h_ref[i] = h[:, i * BR:(i + 1) * BR]
        return carry

    lax.fori_loop(0, RES + 1, head_body, 0)

    def attn_block(t, g, bg, acc, do_k, do_v, opener, closer):
        slot = _mod2(t - 1, NB)
        gcol = col + bg * BR
        mask = jnp.logical_and(gcol >= row * DH, gcol < (row + 1) * DH)
        both = do_k and do_v
        if do_k:
            q = jnp.where(mask, q_ref[t - RES - 1], 0.0).astype(jnp.bfloat16)
        v_buf, v_slot = (vres, t - NBLK - 1) if both else (ring, slot)
        for j in range(NSTEP):
            opener(j)
            cs = pl.ds((j // 2) * 2 * CW, 2 * CW) if both else pl.ds(j * CW, CW)
            if do_k and not (both and j % 2 == 0):
                s_ref[:, cs] += _dot(q, ring[slot, :, cs])
            else:
                part = lax.dot_general(p_ref[g - 1, :, cs], v_buf[v_slot, :, cs],
                                       (((1,), (1,)), ((), ())),
                                       preferred_element_type=jnp.float32)
                if j == 0:
                    o_ref[...] = part
                else:
                    o_ref[...] += part
            closer(j)
        if do_v:
            o = jnp.where(mask, o_ref[...] * linv_ref[g - 1], 0.0).astype(jnp.bfloat16)
            acc = acc + _dot(o, wo_v[_mod2(t - 2, 4)])
        return acc

    def attn_loop(lo, hi, do_k, do_v, acc):
        def body(t, carry):
            g, bg, acc = carry
            acc = attn_block(t, g, bg, acc, do_k, do_v,
                             lambda j: step_open(t, j, lo, hi), lambda j: step_close(t, j, lo, hi))
            last = bg == BPG - 1
            if do_k:
                @pl.when(last)
                def _():
                    s = s_ref[...] * (DH ** -0.5)
                    e = jnp.exp(s - jnp.max(s, axis=-1, keepdims=True))
                    p_ref[g] = e.astype(jnp.bfloat16)
                    linv_ref[g] = jnp.broadcast_to(1.0 / jnp.sum(e, axis=-1, keepdims=True), (GH, BR))
                    s_ref[...] = jnp.zeros_like(s_ref)
            else:
                for ch in range(4):
                    @pl.when(t == T_U2 + 1 + ch)
                    def _():
                        modb_ref[ch] = _dot(sc, wmb_v[:, ch * D:(ch + 1) * D])
            return jnp.where(last, g + 1, g), jnp.where(last, 0, bg + 1), acc

        g0, bg0 = divmod(lo - RES - 1, BPG)
        return lax.fori_loop(lo, hi + 1, body, (jnp.int32(g0), jnp.int32(bg0), acc))[2]

    acc = jnp.zeros((GH, D), jnp.float32)
    attn_loop(RES + 1, NBLK, True, False, acc)
    acc = attn_loop(NBLK + 1, RES + NBLK, True, True, acc)
    acc = attn_loop(RES + NBLK + 1, NT - 1, False, True, acc)
    acc = attn_block(NT, NG, BPG - 1, acc, False, True, lambda j: None, lambda j: None)
    attn = jnp.broadcast_to(jnp.sum(acc, axis=0, keepdims=True), (GH, D))

    tail = tail_copies()
    x1 = x32 + modb_ref[0] * attn
    h2 = (_layernorm(x1) * (1.0 + modb_ref[2]) + modb_ref[1]).astype(jnp.bfloat16)
    gate = _dot(h2, wg_v[...])
    tail[0].wait()
    hh = (gate * _dot(h2, wu_v[...])).astype(jnp.bfloat16)
    hcol = jnp.transpose(jnp.broadcast_to(hh[0:1, F - BR:F].astype(jnp.float32), (BR, BR)))
    for k in range(NTILE):
        piece_op(T_WD, k, T_WD, T_WD, _wait)
    y = jnp.zeros((GH, D), jnp.float32)
    r0, r1 = 0, WD_PRE
    for cp, n in zip(tail[1:], WD_MXU):
        cp.wait()
        r1 += n
        y = y + _dot(hh[:, r0:r1], wd_v[r0:r1, :])
        r0 = r1
    base = x1 + modb_ref[3] * y
    z = jnp.zeros((GH, D), jnp.float32)
    i = 0
    for cp, n in zip(tail[1 + len(WD_MXU):], WD_VPU):
        cp.wait()
        w = wd_v[F - BR + i:F - BR + i + n, :].astype(jnp.float32)
        for r in range(0, n, 8):
            z = z + w[r:r + 8, :] * jnp.concatenate([hcol[i + r:i + r + 8, :]] * (D // BR), axis=1)
        i += n
    out = base[0:1, :] + modb_ref[3][0:1, :] * jnp.sum(z, axis=0, keepdims=True)
    out_ref[...] = out.astype(out_ref.dtype)


@jax.jit
def pallas_adaLN_cond__sliding_block_cached__glu_gated_bilinear__decode_kernel(
    A_x: jax.Array,
    A_k_cache: jax.Array,
    A_v_cache: jax.Array,
    A_wq: jax.Array,
    A_wo: jax.Array,
    B_x: jax.Array,
    B_w_gate: jax.Array,
    B_w_up: jax.Array,
    B_w_down: jax.Array,
    c: jax.Array,
    w_mod: jax.Array,
):
    sk = A_k_cache.shape[2]
    assert A_k_cache.shape == (1, HQ, sk, DH) and min(4096, max(256, sk // 4)) == WIN
    kt = jnp.swapaxes(A_k_cache, 2, 3).reshape(ROWS, sk)
    vt = jnp.swapaxes(A_v_cache, 2, 3).reshape(ROWS, sk)
    bf16, f32 = jnp.bfloat16, jnp.float32
    out = pl.pallas_call(
        _kernel,
        in_specs=[pl.BlockSpec(memory_space=pl.ANY)] * 10,
        out_specs=pl.BlockSpec(memory_space=pltpu.VMEM),
        out_shape=jax.ShapeDtypeStruct((1, D), A_x.dtype),
        scratch_shapes=[
            pltpu.VMEM((1, D), bf16),
            pltpu.VMEM((1, D), bf16),
            pltpu.VMEM((D, 2 * D), bf16),
            pltpu.VMEM((D, 4 * D), bf16),
            pltpu.VMEM((D, ROWS), bf16),
            pltpu.VMEM((4, BR, D), bf16),
            pltpu.VMEM((D, F), bf16),
            pltpu.VMEM((D, F), bf16),
            pltpu.VMEM((F, D), bf16),
            pltpu.VMEM((RES, BR, WIN), bf16),
            pltpu.VMEM((NB, BR, WIN), bf16),
            pltpu.VMEM((D // BR, GH, BR), bf16),
            pltpu.VMEM((NBLK, GH, BR), f32),
            pltpu.VMEM((GH, WIN), f32),
            pltpu.VMEM((NG, GH, WIN), bf16),
            pltpu.VMEM((NG, GH, BR), f32),
            pltpu.VMEM((GH, BR), f32),
            pltpu.VMEM((4, GH, D), f32),
            pltpu.SemaphoreType.DMA((NSEM,)),
        ],
        compiler_params=pltpu.CompilerParams(
            vmem_limit_bytes=96 * 1024 * 1024,
            disable_bounds_checks=True,
            disable_semaphore_checks=True,
        ),
    )(A_x.reshape(1, D), c, w_mod, A_wq, kt, vt, A_wo, B_w_gate, B_w_up, B_w_down)
    return out.reshape(1, 1, D)
```

```python
import jax
import jax.numpy as jnp
from jax import lax
import jax.experimental.pallas as pl
import jax.experimental.pallas.tpu as pltpu

D = 640
HQ = 32
DH = 192
F = 1536
WIN = 4096
EPS = 1e-5
ROWS = HQ * DH
GH = 8
NG = HQ // GH
BR = 128
NBLK = ROWS // BR
BPG = GH * DH // BR
NT = 2 * NBLK
RES = NBLK - BPG
NP = D // 8
HI, LO = 0, 1

TILES = (
    tuple((r, 32, 256, 1024) for r in range(0, BR, 32))
    + tuple((r, 64, c, 512) for c in (1280, 1792) for r in (0, 64))
    + tuple((r, 32, 2304, 1024) for r in range(0, BR, 32))
    + tuple((0, BR, c, 256) for c in (3328, 3584, 3840, 0))
)
NTILE = len(TILES)
NSTEP = NTILE // 2
CW = WIN // NSTEP
AHEAD = 24
NB = 4

T_MA, T_WQ, T_GU, T_WO, T_G2, T_WD = 0, 5, 35, 47, 87, NT - 1
GU1 = (T_WO - T_GU) * NSTEP // 2
U_TAIL = NP - GU1
WD_PRE = 16 * NTILE
WD_MXU = (256, 512, 256, 128)
WD_VPU = (96, 32)
WD_CHUNKS = WD_MXU + WD_VPU

O_KV = 0
O_HI = O_KV + NB * NTILE
O_MISC = O_HI + 2 * NTILE
O_WD = O_MISC + 3
NSEM = O_WD + len(WD_CHUNKS)

assert sorted((r, c) for (r0, rn, c0, cn) in TILES
              for r in range(r0, r0 + rn, 8) for c in range(c0, c0 + cn, 128)) == [
    (r, c) for r in range(0, BR, 8) for c in range(0, WIN, 128)]
assert (T_WQ - T_MA) * NTILE == NP and (T_GU - T_WQ) * NTILE == 6 * NP
assert (T_G2 - T_WO) * 2 == NP and T_WD - T_WO == NBLK and GU1 + (T_WD - T_G2) * NSTEP // 2 == NP
assert WD_PRE + sum(WD_CHUNKS) == F and sum(WD_VPU) == BR
assert AHEAD % 2 == 0 and AHEAD + 2 * NTILE <= NB * NTILE
assert all((i * 10923) >> 16 == i // 6 for i in range(6 * NP))


def _layernorm(x):
    m = jnp.mean(x, axis=-1, keepdims=True)
    xc = x - m
    v = jnp.mean(xc * xc, axis=-1, keepdims=True)
    return xc * lax.rsqrt(v + EPS)


def _dot(a, b):
    return jnp.dot(a, b, preferred_element_type=jnp.float32)


def _rows(start, size):
    return pl.ds(start if isinstance(start, int) else pl.multiple_of(start, 8), size)


def _mod2(i, m):
    return i % m if isinstance(i, int) else jnp.bitwise_and(i, m - 1)


def _divmod6(i):
    q = lax.shift_right_logical(i * 10923, 16)
    return q, i - q * 6


def _when_in(t, a, b, lo, hi, fn):
    if b <= lo or a > hi:
        return
    if a <= lo and hi < b:
        fn()
    elif a <= lo:
        pl.when(t < b)(fn)
    elif hi < b:
        pl.when(t >= a)(fn)
    else:
        pl.when(jnp.logical_and(t >= a, t < b))(fn)


def _start_hi(cp):
    cp.start(priority=HI)


def _start_lo(cp):
    cp.start(priority=LO)


def _wait(cp):
    cp.wait()


def _kernel(x_hbm, c_hbm, wmod_hbm, wq_hbm, kt_hbm, vt_hbm, wo_hbm, wg_hbm, wu_hbm, wd_hbm,
            out_ref,
            x_v, c_v, wma_v, wmb_v, wq_v, wo_v, wg_v, wu_v, wd_v, vres, ring, h_ref, q_ref, s_ref,
            p_ref, linv_ref, o_ref, modb_ref, sems):
    col0 = kt_hbm.shape[1] - WIN
    copy = pltpu.make_async_copy

    def tile_op(t, k, lo, hi, op):
        slot = _mod2(t, NB)
        rt, rn, ct, cn = TILES[k]

        def tile(src, b, dst, i):
            op(copy(src.at[_rows(b * BR + rt, rn), pl.ds(col0 + ct, cn)],
                    dst.at[i, pl.ds(rt, rn), pl.ds(ct, cn)], sems.at[O_KV + slot * NTILE + k]))

        _when_in(t, 0, RES, lo, hi, lambda: tile(vt_hbm, t, vres, t))
        _when_in(t, RES, RES + NBLK, lo, hi, lambda: tile(kt_hbm, t - RES, ring, slot))
        _when_in(t, RES + NBLK, NT, lo, hi, lambda: tile(vt_hbm, t - NBLK, ring, slot))

    def piece_op(t, k, lo, hi, op):
        sem = sems.at[O_HI + _mod2(t, 2) * NTILE + k]
        j, odd = divmod(k, 2)

        def same(src, dst, r, c0, cn):
            rows, cols = _rows(r * 8, 8), pl.ds(c0, cn)
            op(copy(src.at[rows, cols], dst.at[rows, cols], sem))

        def wq_piece():
            r, c = _divmod6((t - T_WQ) * NSTEP + j)
            same(wq_hbm, wq_v, r + jnp.bitwise_and(r, -8) + odd * 8,
                 pl.multiple_of(c * (ROWS // 6), 128), ROWS // 6)

        def half_piece(src, dst, r):
            same(src, dst, r + j // 2, (j % 2) * (F // 2), F // 2)

        def wo_piece():
            op(copy(wo_hbm.at[_rows((t - T_WO) * BR + j * 16, 16)],
                    wo_v.at[_mod2(t, 4), pl.ds(j * 16, 16)], sem))

        def mb_piece():
            rows = _rows((t - T_WO) * 8 + (j % 2) * (D // 2), 8)
            op(copy(wmod_hbm.at[rows, pl.ds((2 + j // 2) * D, D)],
                    wmb_v.at[rows, pl.ds((j // 2) * D, D)], sem))

        def wd_piece():
            op(copy(wd_hbm.at[pl.ds(k * 16, 16)], wd_v.at[pl.ds(k * 16, 16)], sem))

        _when_in(t, T_MA, T_WQ, lo, hi,
                 lambda: same(wmod_hbm, wma_v, (t - T_MA) * NSTEP + j + odd * (NP // 2), 0, 2 * D))
        _when_in(t, T_WQ, T_GU, lo, hi, wq_piece)
        if odd:
            _when_in(t, T_GU, T_WO, lo, hi, lambda: half_piece(wu_hbm, wu_v, (t - T_GU) * 4))
            _when_in(t, T_WO, T_G2, lo, hi, mb_piece)
            _when_in(t, T_G2, T_WD, lo, hi, lambda: half_piece(wg_hbm, wg_v, GU1 + (t - T_G2) * 4))
        else:
            _when_in(t, T_GU, T_WO, lo, hi, lambda: half_piece(wg_hbm, wg_v, (t - T_GU) * 4))
            _when_in(t, T_WO, T_WD, lo, hi, wo_piece)
        _when_in(t, T_WD, NT, lo, hi, wd_piece)

    def tail_copies():
        rows = pl.ds(D - 8 * U_TAIL, 8 * U_TAIL)
        cps = [copy(wu_hbm.at[rows], wu_v.at[rows], sems.at[O_MISC + 2])]
        r = WD_PRE
        for i, n in enumerate(WD_CHUNKS):
            cps.append(copy(wd_hbm.at[pl.ds(r, n)], wd_v.at[pl.ds(r, n)], sems.at[O_WD + i]))
            r += n
        return cps

    def start_tail():
        for cp in tail_copies():
            _start_lo(cp)

    def step_open(t, j, lo, hi):
        tile_op(t, 2 * j, lo, hi, _wait)
        piece_op(t, 2 * j, lo, hi, _start_hi)

    def step_close(t, j, lo, hi):
        db, k = divmod(2 * j + AHEAD, NTILE)
        tile_op(t + db, k, lo + db, hi + db, _start_lo)
        tile_op(t + db, k + 1, lo + db, hi + db, _start_lo)
        if k + 2 == NTILE:
            _when_in(t + db, NT - 1, NT, lo + db, hi + db, start_tail)
        tile_op(t, 2 * j + 1, lo, hi, _wait)
        piece_op(t - 1, 2 * j, lo - 1, hi - 1, _wait)
        piece_op(t - 1, 2 * j + 1, lo - 1, hi - 1, _wait)
        piece_op(t, 2 * j + 1, lo, hi, _start_hi)

    cp_c = copy(c_hbm, c_v, sems.at[O_MISC])
    cp_x = copy(x_hbm, x_v, sems.at[O_MISC + 1])
    for u in range(AHEAD):
        t, k = divmod(u, NTILE)
        tile_op(t, k, t, t, _start_lo)
        if u == 0:
            _start_hi(cp_c)
            _start_hi(cp_x)

    s_ref[...] = jnp.zeros_like(s_ref)
    q_ref[...] = jnp.zeros_like(q_ref)
    cp_c.wait()
    cp_x.wait()
    c32 = jnp.broadcast_to(c_v[...].astype(jnp.float32), (GH, D))
    sc = (c32 * jax.nn.sigmoid(c32)).astype(jnp.bfloat16)
    x32 = jnp.broadcast_to(x_v[...].astype(jnp.float32), (GH, D))
    row = lax.broadcasted_iota(jnp.int32, (GH, BR), 0)
    col = lax.broadcasted_iota(jnp.int32, (GH, BR), 1)

    def head_body(t, carry):
        r, rem = _divmod6(t)
        is_q = jnp.logical_and(rem == 0, t >= 12)
        qb = NBLK // NSTEP
        for j in range(NSTEP):
            step_open(t, j, 0, RES)

            @pl.when(is_q)
            def _():
                res = _dot(h_ref[r - 2],
                           wq_v[_rows((r - 2) * BR, BR), j * qb * BR:(j + 1) * qb * BR])
                for i in range(qb):
                    q_ref[j * qb + i] += res[:, i * BR:(i + 1) * BR]

            step_close(t, j, 0, RES)

        @pl.when(t == T_WQ)
        def _():
            mod_a = _dot(sc, wma_v[...])
            h = (_layernorm(x32) * (1.0 + mod_a[:, D:2 * D]) + mod_a[:, 0:D]).astype(jnp.bfloat16)
            for i in range(D // BR):
                h_ref[i] = h[:, i * BR:(i + 1) * BR]
        return carry

    lax.fori_loop(0, RES + 1, head_body, 0)

    def attn_block(t, g, bg, acc, do_k, do_v, opener, closer):
        slot = _mod2(t - 1, NB)
        gcol = col + bg * BR
        mask = jnp.logical_and(gcol >= row * DH, gcol < (row + 1) * DH)
        both = do_k and do_v
        if do_k:
            q = jnp.where(mask, q_ref[t - RES - 1], 0.0).astype(jnp.bfloat16)
        v_buf, v_slot = (vres, t - NBLK - 1) if both else (ring, slot)
        for j in range(NSTEP):
            opener(j)
            cs = pl.ds((j // 2) * 2 * CW, 2 * CW) if both else pl.ds(j * CW, CW)
            if do_k and not (both and j % 2 == 0):
                s_ref[:, cs] += _dot(q, ring[slot, :, cs])
            else:
                part = lax.dot_general(p_ref[g - 1, :, cs], v_buf[v_slot, :, cs],
                                       (((1,), (1,)), ((), ())),
                                       preferred_element_type=jnp.float32)
                if j == 0:
                    o_ref[...] = part
                else:
                    o_ref[...] += part
            closer(j)
        if do_v:
            o = jnp.where(mask, o_ref[...] * linv_ref[g - 1], 0.0).astype(jnp.bfloat16)
            acc = acc + _dot(o, wo_v[_mod2(t - 2, 4)])
        return acc

    def attn_loop(lo, hi, do_k, do_v, acc):
        def body(t, carry):
            g, bg, acc = carry
            acc = attn_block(t, g, bg, acc, do_k, do_v,
                             lambda j: step_open(t, j, lo, hi), lambda j: step_close(t, j, lo, hi))
            last = bg == BPG - 1
            if do_k:
                @pl.when(last)
                def _():
                    s = s_ref[...] * (DH ** -0.5)
                    e = jnp.exp(s - jnp.max(s, axis=-1, keepdims=True))
                    p_ref[g] = e.astype(jnp.bfloat16)
                    linv_ref[g] = jnp.broadcast_to(1.0 / jnp.sum(e, axis=-1, keepdims=True), (GH, BR))
                    s_ref[...] = jnp.zeros_like(s_ref)
            else:
                for ch in range(4):
                    @pl.when(t == T_G2 + 1 + ch)
                    def _():
                        modb_ref[ch] = _dot(sc, wmb_v[:, ch * D:(ch + 1) * D])
            return jnp.where(last, g + 1, g), jnp.where(last, 0, bg + 1), acc

        g0, bg0 = divmod(lo - RES - 1, BPG)
        return lax.fori_loop(lo, hi + 1, body, (jnp.int32(g0), jnp.int32(bg0), acc))[2]

    acc = jnp.zeros((GH, D), jnp.float32)
    attn_loop(RES + 1, NBLK, True, False, acc)
    acc = attn_loop(NBLK + 1, RES + NBLK, True, True, acc)
    acc = attn_loop(RES + NBLK + 1, NT - 1, False, True, acc)
    acc = attn_block(NT, NG, BPG - 1, acc, False, True, lambda j: None, lambda j: None)
    attn = jnp.broadcast_to(jnp.sum(acc, axis=0, keepdims=True), (GH, D))

    tail = tail_copies()
    x1 = x32 + modb_ref[0] * attn
    h2 = (_layernorm(x1) * (1.0 + modb_ref[2]) + modb_ref[1]).astype(jnp.bfloat16)
    gate = _dot(h2, wg_v[...])
    tail[0].wait()
    hh = (gate * _dot(h2, wu_v[...])).astype(jnp.bfloat16)
    hcol = jnp.transpose(jnp.broadcast_to(hh[0:1, F - BR:F].astype(jnp.float32), (BR, BR)))
    for k in range(NTILE):
        piece_op(T_WD, k, T_WD, T_WD, _wait)
    y = jnp.zeros((GH, D), jnp.float32)
    r0, r1 = 0, WD_PRE
    for cp, n in zip(tail[1:], WD_MXU):
        cp.wait()
        r1 += n
        y = y + _dot(hh[:, r0:r1], wd_v[r0:r1, :])
        r0 = r1
    base = x1 + modb_ref[3] * y
    z = jnp.zeros((GH, D), jnp.float32)
    i = 0
    for cp, n in zip(tail[1 + len(WD_MXU):], WD_VPU):
        cp.wait()
        w = wd_v[F - BR + i:F - BR + i + n, :].astype(jnp.float32)
        for r in range(0, n, 8):
            z = z + w[r:r + 8, :] * jnp.concatenate([hcol[i + r:i + r + 8, :]] * (D // BR), axis=1)
        i += n
    out = base[0:1, :] + modb_ref[3][0:1, :] * jnp.sum(z, axis=0, keepdims=True)
    out_ref[...] = out.astype(out_ref.dtype)


@jax.jit
def pallas_adaLN_cond__sliding_block_cached__glu_gated_bilinear__decode_kernel(
    A_x: jax.Array,
    A_k_cache: jax.Array,
    A_v_cache: jax.Array,
    A_wq: jax.Array,
    A_wo: jax.Array,
    B_x: jax.Array,
    B_w_gate: jax.Array,
    B_w_up: jax.Array,
    B_w_down: jax.Array,
    c: jax.Array,
    w_mod: jax.Array,
):
    sk = A_k_cache.shape[2]
    assert A_k_cache.shape == (1, HQ, sk, DH) and min(4096, max(256, sk // 4)) == WIN
    kt = jnp.swapaxes(A_k_cache, 2, 3).reshape(ROWS, sk)
    vt = jnp.swapaxes(A_v_cache, 2, 3).reshape(ROWS, sk)
    bf16, f32 = jnp.bfloat16, jnp.float32
    out = pl.pallas_call(
        _kernel,
        in_specs=[pl.BlockSpec(memory_space=pl.ANY)] * 10,
        out_specs=pl.BlockSpec(memory_space=pltpu.VMEM),
        out_shape=jax.ShapeDtypeStruct((1, D), A_x.dtype),
        scratch_shapes=[
            pltpu.VMEM((1, D), bf16),
            pltpu.VMEM((1, D), bf16),
            pltpu.VMEM((D, 2 * D), bf16),
            pltpu.VMEM((D, 4 * D), bf16),
            pltpu.VMEM((D, ROWS), bf16),
            pltpu.VMEM((4, BR, D), bf16),
            pltpu.VMEM((D, F), bf16),
            pltpu.VMEM((D, F), bf16),
            pltpu.VMEM((F, D), bf16),
            pltpu.VMEM((RES, BR, WIN), bf16),
            pltpu.VMEM((NB, BR, WIN), bf16),
            pltpu.VMEM((D // BR, GH, BR), bf16),
            pltpu.VMEM((NBLK, GH, BR), f32),
            pltpu.VMEM((GH, WIN), f32),
            pltpu.VMEM((NG, GH, WIN), bf16),
            pltpu.VMEM((NG, GH, BR), f32),
            pltpu.VMEM((GH, BR), f32),
            pltpu.VMEM((4, GH, D), f32),
            pltpu.SemaphoreType.DMA((NSEM,)),
        ],
        compiler_params=pltpu.CompilerParams(
            vmem_limit_bytes=96 * 1024 * 1024,
            disable_bounds_checks=True,
            disable_semaphore_checks=True,
        ),
    )(A_x.reshape(1, D), c, w_mod, A_wq, kt, vt, A_wo, B_w_gate, B_w_up, B_w_down)
    return out.reshape(1, 1, D)
```
